```python
import jax
import jax.numpy as jnp

def _softmax(x, axis=-1):
    return jax.nn.softmax(x, axis=axis)

def _gelu(x):
    return jax.nn.gelu(x, approximate=True)

def _silu(x):
    return jax.nn.silu(x)

def _sigmoid(x):
    return jax.nn.sigmoid(x)

def _layernorm(x, axis=-1, eps=1e-05):
    m = jnp.mean(x, axis=axis, keepdims=True)
    v = jnp.var(x, axis=axis, keepdims=True)
    return (x - m) / jnp.sqrt(v + eps)

def _scatter_add(tgt, idx, src, axis=0):
    return tgt.at[idx].add(src)

def _segment_sum(src, seg, n):
    return jax.ops.segment_sum(src, seg, n)

class _Rng:

    def __init__(self, key):
        self._k = key

    def _next(self):
        self._k, sub = jax.random.split(self._k)
        return sub

    def normal(self, shape):
        return jax.random.normal(self._next(), shape, dtype=jnp.bfloat16)

    def randint(self, lo, hi, shape):
        return jax.random.randint(self._next(), shape, lo, hi, dtype=jnp.int32)

    def uniform(self, shape, lo=0.0, hi=1.0):
        return jax.random.uniform(self._next(), shape, jnp.bfloat16, lo, hi)

    def permutation(self, n):
        return jax.random.permutation(self._next(), n)
kernel_name = 'interleave_layers__memory_aug_infini_attn__sliding_local_dilated__prompt'

def setup_inputs():
    _rng = _Rng(jax.random.key(int.from_bytes(__import__("os").urandom(4), "little")))
    _w = lambda a: (lambda t: t.astype(jnp.bfloat16) if jnp.issubdtype(t.dtype, jnp.floating) else t)(jnp.asarray(a))

    def _A_setup():
        B, S, D, H = (1, 2048, 1024, 32)
        N = 4
        L = max(1, S // N)
        sc = D ** (-0.5)
        return {'x': _w((lambda *s: _rng.normal(s) * 0.05)(B, N * L, D)), 'wq': _w((lambda *s: _rng.normal(s) * 0.05)(D, D) * sc), 'wk': _w((lambda *s: _rng.normal(s) * 0.05)(D, D) * sc), 'wv': _w((lambda *s: _rng.normal(s) * 0.05)(D, D) * sc), 'wo': _w((lambda *s: _rng.normal(s) * 0.05)(D, D) * sc), 'beta': _w((lambda *s: _rng.normal(s) * 0.05)(H))}
    _A_in = _A_setup()

    def _B_setup():
        B, S, D = (1, 2048, 1024)
        return {'x': _w((lambda *s: _rng.normal(s) * 0.05)(B, S, D)), 'wqkv': _w((lambda *s: _rng.normal(s) * 0.05)(D, 3 * D)), 'wo': _w((lambda *s: _rng.normal(s) * 0.05)(D, D))}
    _B_in = _B_setup()
    return {'A_x': _A_in['x'], 'A_wq': _A_in['wq'], 'A_wk': _A_in['wk'], 'A_wv': _A_in['wv'], 'A_wo': _A_in['wo'], 'A_beta': _A_in['beta'], 'B_x': _B_in['x'], 'B_wqkv': _B_in['wqkv'], 'B_wo': _B_in['wo']}

def reference(A_x, A_wq, A_wk, A_wv, A_wo, A_beta, B_x, B_wqkv, B_wo):

    def _A_ref(x, wq, wk, wv, wo, beta):
        B, S, D = x.shape
        H = 32
        Dh = D // H
        N = 4
        L = S // N
        q = (lambda x, *d: x.transpose(*d))((x @ wq).reshape(B, S, H, Dh), 0, 2, 1, 3).reshape(B, H, N, L, Dh)
        k = (lambda x, *d: x.transpose(*d))((x @ wk).reshape(B, S, H, Dh), 0, 2, 1, 3).reshape(B, H, N, L, Dh)
        v = (lambda x, *d: x.transpose(*d))((x @ wv).reshape(B, S, H, Dh), 0, 2, 1, 3).reshape(B, H, N, L, Dh)
        phi = lambda t: jnp.where(t > 0, t + 1.0, jnp.exp(t))
        scale = Dh ** (-0.5)
        ar = jnp.arange(L)
        mask = (lambda x, dt: x.astype(dt))(ar[:, None] < ar[None, :], x.dtype) * -1000000000.0
        g = _sigmoid(beta).reshape(1, H, 1, 1)
        M = jnp.einsum('bhd,bhe->bhde', q[:, :, 0, 0, :] * 0.0, q[:, :, 0, 0, :] * 0.0)
        z = q[:, :, 0, 0, :] * 0.0
        outs = []
        for s in range(N):
            qs, ks, vs = (q[:, :, s].copy(), k[:, :, s].copy(), v[:, :, s].copy())
            logits = jnp.einsum('bhqd,bhkd->bhqk', qs, ks) * scale + mask
            p = _softmax(logits, axis=-1)
            a_dot = jnp.einsum('bhqk,bhkd->bhqd', p, vs)
            pq = phi(qs)
            num = jnp.einsum('bhld,bhde->bhle', pq, M)
            den = jnp.einsum('bhld,bhd->bhl', pq, z)[..., None] + 1e-06
            a_mem = num / den
            o = g * a_mem + (1.0 - g) * a_dot
            outs.append(o)
            pk = phi(ks)
            M = M + jnp.einsum('bhld,bhle->bhde', pk, vs)
            z = z + jnp.einsum('bhld->bhd', pk)
        o = (lambda x, *d: x.transpose(*d))(jnp.stack(outs, 2).reshape(B, H, S, Dh), 0, 2, 1, 3).reshape(B, S, D)
        return o @ wo

    def _B_ref(x, wqkv, wo):
        B, S, D = x.shape
        H = 32
        Dh = D // H
        W, dil = (8, 2)
        qkv = (lambda x, *d: x.transpose(*d))((x @ wqkv).reshape(B, S, 3, H, Dh), 2, 0, 3, 1, 4)
        q, k, v = (qkv[0], qkv[1], qkv[2])
        scale = Dh ** (-0.5)
        pos = jnp.arange(S)
        off = jnp.arange(W) * dil
        idx = pos[:, None] - off[None, :]
        mask = idx >= 0
        idx_c = jnp.where(mask, idx, 0).reshape(-1)
        kg = k[:, :, idx_c, :].reshape(B, H, S, W, Dh)
        vg = v[:, :, idx_c, :].reshape(B, H, S, W, Dh)
        logits = jnp.einsum('bhsd,bhswd->bhsw', q, kg) * scale
        logits = jnp.where(mask[None, None, :, :], logits, -1000000000.0)
        attn = _softmax(logits, axis=-1)
        o = jnp.einsum('bhsw,bhswd->bhsd', attn, vg)
        return (lambda x, *d: x.transpose(*d))(o, 0, 2, 1, 3).reshape(B, S, D) @ wo
    x = A_x
    x = x + _A_ref(_layernorm(x, axis=-1), A_wq, A_wk, A_wv, A_wo, A_beta)
    x = x + _B_ref(_layernorm(x, axis=-1), B_wqkv, B_wo)
    x = x + _A_ref(_layernorm(x, axis=-1), A_wq, A_wk, A_wv, A_wo, A_beta)
    x = x + _B_ref(_layernorm(x, axis=-1), B_wqkv, B_wo)
    return x
```

```python
import functools
import math

import jax
import jax.numpy as jnp
from jax import lax
import jax.experimental.pallas as pl
import jax.experimental.pallas.tpu as pltpu

S, D, H, DH = 2048, 1024, 32, 32
NSEG, L = 4, 512
G = 8
WIN, DIL = 8, 2
HALO = 16
LOG2E = math.log2(math.e)
QSCALE = DH ** -0.5 * LOG2E
NEG = -1e30
F32, BF16, I32 = jnp.float32, jnp.bfloat16, jnp.int32
NN = (((1,), (0,)), ((), ()))
NT = (((1,), (1,)), ((), ()))

CFG = dict(prow=128, orow=128)


def _dot(a, b, dims=NN):
    return lax.dot_general(a, b, dims, preferred_element_type=F32)


def _iota(shape, axis):
    return lax.broadcasted_iota(I32, shape, axis)


def _phi(t):
    return jnp.where(t > 0, t + 1.0, jnp.exp(t))


def _layernorm(x):
    m = jnp.mean(x, axis=-1, keepdims=True)
    c = x - m
    v = jnp.mean(c * c, axis=-1, keepdims=True)
    return c * lax.rsqrt(v + 1e-5)


def _run(order, **streams):
    for name in order:
        next(streams[name], None)
    for st in streams.values():
        for _ in st:
            pass


def _kernel(x_hbm, wq_hbm, wk_hbm, wv_hbm, woa_hbm, beta_ref, wqkv_hbm, wob_hbm,
            out_hbm,
            xio, xres, xn, wa, woa, wb, wob, qkv0, qkv1, obuf, mem, gate,
            kvn, kvt, halo, otmp, sems, osems):
    qkvs = (qkv0, qkv1)
    prow, orow = CFG["prow"], CFG["orow"]

    copies = []
    for s in range(NSEG):
        copies.append(pltpu.make_async_copy(x_hbm.at[pl.ds(s * L, L)], xio.at[s], sems.at[s]))
    for i, w in enumerate((wq_hbm, wk_hbm, wv_hbm)):
        copies.append(pltpu.make_async_copy(w, wa.at[:, pl.ds(i * D, D)], sems.at[4 + i]))
    copies.append(pltpu.make_async_copy(woa_hbm, woa, sems.at[7]))
    copies.append(pltpu.make_async_copy(wqkv_hbm, wb, sems.at[8]))
    copies.append(pltpu.make_async_copy(wob_hbm, wob, sems.at[9]))
    for c in copies:
        c.start()

    b = jnp.broadcast_to(beta_ref[...].astype(F32), (H, H))
    b = jnp.sum(jnp.where(_iota((H, H), 0) == _iota((H, H), 1), b, 0.0), axis=1, keepdims=True)
    gate[...] = jnp.broadcast_to(1.0 / (1.0 + jnp.exp(-b)), (H, 128))

    for c in copies:
        c.wait()

    for r in range(0, L, 64):
        x = xio[0, r:r + 64, :].astype(F32)
        xres[0, r:r + 64, :] = x
        xn[r:r + 64, :] = _layernorm(x).astype(BF16)

    def proj(w, g):
        dst = qkvs[g % 2]
        for c in range(3):
            for r in range(0, L, prow):
                col = c * D + g * 128
                dst[c, r:r + prow, :] = _dot(xn[r:r + prow, :], w[:, col:col + 128])
                yield

    def out_proj(w, s, k0, k1, last):
        for r in range(0, L, orow):
            for c in range(0, D, 512):
                y = xres[s, r:r + orow, c:c + 512] + _dot(obuf[r:r + orow, k0:k1], w[k0:k1, c:c + 512])
                xres[s, r:r + orow, c:c + 512] = y
                if last:
                    xio[s, r:r + orow, c:c + 512] = y.astype(BF16)
                yield

    def norm_next(sn, from_input):
        for r in range(0, L, 64):
            x = xres[sn, r:r + 64, :]
            if from_input is not None:
                x = jnp.where(from_input, xio[sn, r:r + 64, :].astype(F32), x)
                xres[sn, r:r + 64, :] = x
            xn[r:r + 64, :] = _layernorm(x).astype(BF16)
            yield

    def attn_a(g, s):
        src = qkvs[g % 2]
        lane_head = _iota((128, 128), 1) // DH
        causal = _iota((128, 128), 0) <= _iota((128, 128), 1)
        k = src[1]
        kb = k.astype(BF16)
        vt = src[2].T.astype(BF16)
        yield

        def qk(i):
            q = src[0, i * 128:(i + 1) * 128, :] * QSCALE
            qm = jnp.concatenate(
                [jnp.where(lane_head == h, q, 0.0).astype(BF16) for h in range(4)], axis=0)
            return _dot(kb[:(i + 1) * 128], qm, NT)

        def softmax(st, i):
            ps, ls = [], []
            for h in range(4):
                sh = st[:, h * 128:(h + 1) * 128]
                diag = jnp.where(causal, sh[i * 128:], NEG)
                sh = jnp.concatenate([sh[:i * 128], diag], axis=0) if i else diag
                p = jnp.exp2(sh - jnp.max(sh, axis=0, keepdims=True))
                ls.append(jnp.sum(p, axis=0, keepdims=True))
                ps.append(p.astype(BF16))
            return ps, ls

        def pv(ps, ls, i):
            n = (i + 1) * 128
            pq = _phi(src[0, i * 128:(i + 1) * 128, :]).astype(BF16)
            nd = _dot(mb, pq, NT)
            outs = []
            for h in range(4):
                gh = gate[4 * g + h:4 * g + h + 1, :]
                a = _dot(vt[h * DH:(h + 1) * DH, :n], ps[h])
                den = nd[128 + h:129 + h] + 1e-6
                outs.append(nd[h * DH:(h + 1) * DH] * (gh / den) + a * ((1.0 - gh) / ls[h]))
            o = jnp.concatenate(outs, axis=0).T
            obuf[i * 128:(i + 1) * 128, g * 128:(g + 1) * 128] = o.astype(BF16)

        m_old = jnp.where(s > 0, mem[g], 0.0)
        mb = m_old.astype(BF16)
        prev = None
        for i in (3, 2, 1, 0):
            if prev is not None:
                pv(*prev)
            st = qk(i)
            prev = softmax(st, i) + (i,)
            yield
        pv(*prev)
        pk = _phi(k)
        upd = _dot(vt, pk.astype(BF16))
        z = jnp.sum(pk, axis=0, keepdims=True)
        mem[g, :128, :] = m_old[:128] + jnp.where(_iota((128, 128), 0) // DH == lane_head, upd, 0.0)
        mem[g, 128:, :] = m_old[128:] + jnp.where(_iota((16, 128), 0) == lane_head[:16], z, 0.0)
        yield

    def attn_b(g, s):
        src = qkvs[g % 2]
        sub = _iota((8, 128), 0)
        bits = [(sub & b) != 0 for b in (1, 2, 4)]

        def rnd(t):
            return lax.bitcast_convert_type(t.astype(BF16).astype(F32), I32)

        kvn[:HALO, :] = jnp.where(s > 0, halo[g], 0)
        kv = rnd(src[1]) | lax.shift_right_logical(rnd(src[2]), 16)
        kvn[HALO:, :] = kv
        halo[g] = kv[L - HALO:]
        yield
        for par in range(2):
            ms = list(range(par - 14, par + 3, 2))
            for n, m in enumerate(ms):
                kvt[par, n] = kvn[pl.ds(HALO + m, 128, stride=4), :].T
            qts = [(src[0, pl.ds(j, 128, stride=4), :] * QSCALE).T for j in (par, par + 2)]
            valid = [s * L + 4 * _iota((8, 128), 1) + j - DIL * sub >= 0 for j in (par, par + 2)]
            yield
            outs = [[], []]
            for h in range(4):
                rows = slice(h * DH, (h + 1) * DH)
                part = [[None] * WIN, [None] * WIN]
                for n in range(len(ms)):
                    kk = lax.bitcast_convert_type(kvt[par, n, rows, :] & -65536, F32)
                    for a in range(2):
                        w = 7 + a - n
                        if 0 <= w < WIN:
                            t = qts[a][rows] * kk
                            part[a][w] = (t[0:8] + t[8:16]) + (t[16:24] + t[24:32])
                probs = []
                for a in range(2):
                    cur = part[a]
                    for bit, sh in zip(bits, (1, 2, 4)):
                        cur = [jnp.where(bit, y, x) + pltpu.roll(jnp.where(bit, x, y), sh, 0)
                               for x, y in zip(cur[0::2], cur[1::2])]
                    lg = jnp.where(valid[a], cur[0], NEG)
                    p = jnp.exp2(lg - jnp.max(lg, axis=0, keepdims=True))
                    probs.append(p / jnp.sum(p, axis=0, keepdims=True))
                acc = [None, None]
                for n in range(len(ms)):
                    vv = lax.bitcast_convert_type(kvt[par, n, rows, :] << 16, F32)
                    for a in range(2):
                        w = 7 + a - n
                        if 0 <= w < WIN:
                            t = probs[a][w:w + 1] * vv
                            acc[a] = t if acc[a] is None else acc[a] + t
                for a in range(2):
                    outs[a].append(acc[a])
                yield
            for a in range(2):
                otmp[pl.ds(par + 2 * a, 128, stride=4), :] = jnp.concatenate(outs[a], axis=0).T
        obuf[:, g * 128:(g + 1) * 128] = otmp[...].astype(BF16)
        yield

    def layer(attn, order, w, wo, s, from_input, last):
        _run("", p=proj(w, 0))
        for g in range(G - 1):
            _run(order, t=attn(g, s), p=proj(w, g + 1))
        _run(CFG["order_last"][attn is attn_b], t=attn(G - 1, s), p=out_proj(wo, s, 0, 512, False))
        _run("np" * 8, n=norm_next((s + 1) % NSEG, from_input), p=out_proj(wo, s, 512, D, last))

    def out_copy(s):
        return pltpu.make_async_copy(xio.at[s], out_hbm.at[pl.ds(pl.multiple_of(s * L, L), L)], osems.at[s])

    def pair(rep, _):
        def a_body(s, _):
            layer(attn_a, CFG["order_a"], wa, woa, s, jnp.logical_and(rep == 0, s < NSEG - 1), False)

        def b_body(s, _):
            layer(attn_b, CFG["order_b"], wb, wob, s, None, True)

            @pl.when(rep == 1)
            def _():
                out_copy(s).start()

        lax.fori_loop(0, NSEG, a_body, None)
        lax.fori_loop(0, NSEG, b_body, None)

    lax.fori_loop(0, 2, pair, None)
    for s in range(NSEG):
        pltpu.make_async_copy(xio.at[s], out_hbm.at[pl.ds(s * L, L)], osems.at[s]).wait()


CFG["order_a"] = "tpptpptpptpptptppp"
CFG["order_b"] = "tp" * 12
CFG["order_last"] = ("tptptptptptppp", "ttpttptptpttptptptp")


def build(interpret=False):
    any_spec = pl.BlockSpec(memory_space=pl.ANY)
    return pl.pallas_call(
        _kernel,
        out_shape=jax.ShapeDtypeStruct((S, D), BF16),
        in_specs=[any_spec] * 5 + [pl.BlockSpec(memory_space=pltpu.VMEM)] + [any_spec] * 2,
        out_specs=any_spec,
        scratch_shapes=[
            pltpu.VMEM((NSEG, L, D), BF16),
            pltpu.VMEM((NSEG, L, D), F32),
            pltpu.VMEM((L, D), BF16),
            pltpu.VMEM((D, 3 * D), BF16),
            pltpu.VMEM((D, D), BF16),
            pltpu.VMEM((D, 3 * D), BF16),
            pltpu.VMEM((D, D), BF16),
            pltpu.VMEM((3, L, 128), F32),
            pltpu.VMEM((3, L, 128), F32),
            pltpu.VMEM((L, D), BF16),
            pltpu.VMEM((G, 144, 128), F32),
            pltpu.VMEM((H, 128), F32),
            pltpu.VMEM((HALO + L, 128), I32),
            pltpu.VMEM((2, 9, 128, 128), I32),
            pltpu.VMEM((G, HALO, 128), I32),
            pltpu.VMEM((L, 128), F32),
            pltpu.SemaphoreType.DMA((10,)),
            pltpu.SemaphoreType.DMA((NSEG,)),
        ],
        compiler_params=pltpu.CompilerParams(vmem_limit_bytes=100 * 2 ** 20),
        interpret=interpret,
        name="fused",
    )


@jax.jit
def pallas_interleave_layers__memory_aug_infini_attn__sliding_local_dilated__prompt_kernel(A_x, A_wq, A_wk, A_wv, A_wo, A_beta, B_x, B_wqkv, B_wo):
    del B_x
    out = build()(A_x.reshape(S, D), A_wq, A_wk, A_wv, A_wo, A_beta.reshape(1, H), B_wqkv, B_wo)
    return out.reshape(A_x.shape)
```

```python
import contextlib
import math

import jax
import jax.numpy as jnp
from jax import lax
import jax.experimental.pallas as pl
import jax.experimental.pallas.tpu as pltpu

S, D, H, DH = 2048, 1024, 32, 32
NSEG, L = 4, 512
HL = L // 2
NPAIR = 4
NUNIT = 16
WIN, DIL = 8, 2
HALO = 16
LOG2E = math.log2(math.e)
QSCALE = DH ** -0.5 * LOG2E
NEG = -1e9 * LOG2E
F32, BF16, I32 = jnp.float32, jnp.bfloat16, jnp.int32

CFG = dict(prow=128, orow=64, only=None, steps_a=2, steps_b=2, flags={}, tick=True, due=True, slack=4)


def _scope(name):
    return jax.named_scope(name) if CFG.get("scopes") else contextlib.nullcontext()


def _dot(a, b):
    return jnp.dot(a, b, preferred_element_type=F32)


def _iota(shape, axis):
    return lax.broadcasted_iota(I32, shape, axis)


def _pk(x):
    return pltpu.bitcast(x.astype(BF16), I32)


def _upk(x):
    return pltpu.bitcast(x, BF16)


def _half(start, size):
    return slice(start // 2, (start + size) // 2)


def _blk(i, n=128):
    return slice(i * n, (i + 1) * n)


def _token(half, r):
    return r // 64 * 128 + half * 64 + r % 64


def _phi(t):
    return jnp.where(t > 0, t + 1.0, jnp.exp(t))


def _lhs_terms(a11, a12, a21, a22):
    return (a11 + a22, a21 + a22, a11, a22, a11 + a12, a21 - a11, a12 - a22)


def _rhs_terms(b11, b12, b21, b22):
    return (b11 + b22, b11, b12 - b22, b21 - b11, b22, b11 + b12, b21 + b22)


def _strassen(prod, emit):
    m = prod(0)
    c11 = c22 = m
    yield m
    m = prod(6)
    c11 = c11 + m
    yield m
    m = prod(5)
    c22 = c22 + m
    yield m
    c21 = prod(3)
    c11 = c11 + c21
    yield c21
    m = prod(1)
    c22 = c22 - m
    emit(1, 0, c21 + m)
    yield m
    c12 = prod(4)
    emit(0, 0, c11 - c12)
    yield c12
    m = prod(2)
    emit(1, 1, c22 + m)
    emit(0, 1, c12 + m)
    yield m


def _drain(gen):
    for _ in gen:
        pass


def _weave(main, tasks, pace):
    tasks = sorted(tasks, key=lambda t: t[0])
    pace.clear()
    k = 0
    while k < len(tasks) and tasks[k][0] < 0:
        tasks[k][1]()
        k += 1
    for i, m in enumerate(main):
        while k < len(tasks) and tasks[k][0] < i + 1:
            r = int((tasks[k][0] - i) * m.shape[0]) // 8 * 8
            pace["rows"] = m[r:r + 8]
            tasks[k][1]()
            k += 1
    for _, thunk in tasks[k:]:
        thunk()
    pace.clear()


def _spread(start, length, thunks):
    return [(start + length * k / len(thunks), f) for k, f in enumerate(thunks)]


def _kernel(x_hbm, wq_hbm, wk_hbm, wv_hbm, woa_hbm, beta_ref, wqkv_hbm, wob_hbm,
            out_hbm,
            xio, xres, xtmp, xs, os_, wraw, wst, q0, k0, v0, q1, k1, v1, mem, gate, cmask,
            halo, xsem, wsem, osem, *bufs):
    bufs = list(bufs)
    kvn, otmp = ([bufs.pop(0) for _ in range(2)] for _ in range(2))
    abuf, sbuf, kvt, otr = ([[bufs.pop(0) for _ in range(k)] for _ in range(2)] for k in (4, 4, 2, 2))
    pace = {}
    never = [None]
    qkvs = ((q0, k0, v0), (q1, k1, v1))
    prow, orow = CFG["prow"], CFG["orow"]

    def x_copy(s):
        return pltpu.make_async_copy(x_hbm.at[pl.ds(pl.multiple_of(s * L, L), L)], xio.at[s], xsem.at[s])

    def w_copy(u):
        t, v = divmod(u, NUNIT)
        if v >= 12:
            src, col = (woa_hbm, wob_hbm)[t], (v - 12) * 256
        elif t == 0:
            src, col = (wq_hbm, wk_hbm, wv_hbm)[v % 3], (v // 3) * 256
        else:
            src, col = wqkv_hbm, (v % 3) * D + (v // 3) * 256
        return pltpu.make_async_copy(src.at[:, pl.ds(col, 256)], wraw.at[u], wsem.at[u])

    def start(units):
        for u in units:
            w_copy(u).start()

    x_copy(0).start()
    start(range(3))
    x_copy(1).start()

    b = jnp.broadcast_to(beta_ref[...].astype(F32), (H, H))
    b = jnp.sum(jnp.where(_iota((H, H), 0) == _iota((H, H), 1), b, 0.0), axis=1, keepdims=True)
    gate[...] = jnp.broadcast_to(1.0 / (1.0 + jnp.exp(-b)), (H, 128))
    cmask[...] = jnp.where(_iota((128, 128), 0) <= _iota((128, 128), 1), 0.0, NEG)

    def paced(x):
        if "rows" not in pace or not CFG["tick"]:
            return x
        rows = lax.bitcast_convert_type(pace["rows"], x.dtype)
        return jnp.where(never[0], jnp.tile(rows, (x.shape[0] // 8, 1)), x)

    def flipped(x):
        return jnp.concatenate([paced(x[:8]), x[8:]], axis=0).T

    def prep(u):
        for t in range(4):
            for r in range(0, 128, 32):
                top = wraw[u, 256 * t + r:256 * t + r + 32, :].astype(F32)
                bot = wraw[u, 256 * t + 128 + r:256 * t + 128 + r + 32, :].astype(F32)
                terms = _rhs_terms(top[:, :128], top[:, 128:], bot[:, :128], bot[:, 128:])
                for i, term in enumerate(terms):
                    wst[u, i, _half(128 * t + r, 32), :] = _pk(term)

    def norm(sn, slot, zr, start, step, lag):
        st = {}

        def mean(r):
            x = xres[sn, r:r + 16, :]
            xtmp[3 * zr, r:r + 16, :] = x
            acc = paced(x[:, :128])
            for t in range(1, 8):
                acc = acc + x[:, _blk(t)]
            st["m", r] = jnp.broadcast_to(jnp.sum(acc, axis=1, keepdims=True) * (1.0 / D), (16, 128))

        def scale(r):
            m = paced(st["m", r])
            acc = None
            for t in range(8):
                c = xtmp[zr, r:r + 16, _blk(t)] - m
                acc = c * c if acc is None else acc + c * c
            var = jnp.sum(acc, axis=1, keepdims=True) * (1.0 / D)
            st["r", r] = jnp.broadcast_to(lax.rsqrt(var + 1e-5), (16, 128))

        def operands(r, t):
            ys = []
            for r0 in (_token(0, r), _token(1, r)):
                m = paced(st["m", r0])
                ys += [(xtmp[2 * zr, r0:r0 + 16, _blk(2 * t + k)] - m) * st["r", r0] for k in range(2)]
            for i, term in enumerate(_lhs_terms(*ys)):
                pace["due"] = xs[slot, i, _half(r, 16), _blk(t)] = _pk(term)

        tasks = []
        for k, r in enumerate(range(0, HL, 16)):
            t0 = start + k * step
            rows = (_token(0, r), _token(1, r))
            tasks += _spread(t0, step, [lambda r0=r0: mean(r0) for r0 in rows])
            tasks += _spread(t0 + lag, step, [lambda r0=r0: scale(r0) for r0 in rows])
            tasks += _spread(t0 + 2 * lag + step / 2, step, [lambda r=r, t=t: operands(r, t) for t in range(4)])
        return tasks

    def weights(u, i):
        w = wst[u, i]
        due = pace.setdefault("queue", [])
        due.append(pace.pop("due", None))
        if len(due) > CFG["slack"]:
            last = due.pop(0)
            if last is not None and CFG["due"]:
                w = jnp.concatenate([jnp.where(never[0], lax.bitcast_convert_type(last, I32), w[:8]), w[8:]], axis=0)
        return _upk(w)

    def proj(slot, u0, dst, zw):
        for c in range(3):
            for r in range(0, HL, prow):
                def prod(i):
                    return _dot(_upk(xs[slot, i, _half(r, prow), :]), weights(u0 + c, i))

                def emit(bi, bj, val):
                    for k in range(0, prow, 64):
                        dst[c][zw + bj, pl.ds(_token(bi, r + k), 64), :] = val[k:k + 64]

                yield from _strassen(prod, emit)

    def out_proj(u0, s):
        for v in range(4):
            for r in range(0, HL, orow):
                def prod(i):
                    lhs = jnp.concatenate([os_[t, i, r:r + orow, :] for t in range(4)], axis=1)
                    return _dot(lhs, weights(u0 + v, i))

                def emit(bi, bj, val):
                    for k in range(0, orow, 64):
                        rows = pl.ds(_token(bi, r + k), 64)
                        y = xres[s, rows, _blk(2 * v + bj)] + val[k:k + 64]
                        xres[s, rows, _blk(2 * v + bj)] = y
                        xio[s, rows, _blk(2 * v + bj)] = y.astype(BF16)

                yield from _strassen(prod, emit)

    def put_o(p, r, nr, zr):
        top, bot = pl.ds(_token(0, r), nr), pl.ds(_token(1, r), nr)
        terms = _lhs_terms(paced(otmp[0][zr, top]), otmp[1][zr, top], otmp[0][zr, bot], paced(otmp[1][zr, bot]))
        for i, term in enumerate(terms):
            os_[p, i, r:r + nr, :] = term.astype(BF16)

    def ready(j):
        return [-1 if j == 0 else 42 * (j - 1) + 14 * (c + 1) - 0.01 for c in range(3)]

    def attn_a(src, p, s, zr, zw, j):
        tasks = []
        for e in range(2):
            tasks += attn_a_group(src, p, e, 2 * p + e, s, zr, zw, CFG["a"]["t0"][2 * j + e], ready(j))
        return tasks

    def attn_a_group(src, p, e, g, s, zr, zw, t0, ready):
        st = {}
        KB, VT, QT, PQ = range(4)

        def prepare_q(i):
            qt = flipped(src[0][zr + e, _blk(i), :])
            abuf[e][QT][zw, i] = _pk(qt * QSCALE)
            abuf[e][PQ][zw, i] = _pk(_phi(qt))

        def prepare_k(i):
            abuf[e][KB][zw, i] = _pk(paced(src[1][zr + e, _blk(i), :]))

        def prepare_v(i):
            abuf[e][VT][zw, i] = _pk(flipped(src[2][zr + e, _blk(i), :]))

        def wide(which):
            return _upk(jnp.concatenate([abuf[e][which][zr, i] for i in range(4)], axis=1))

        def retrieve():
            st["m"] = jnp.where(s > 0, mem[g], 0.0)
            st["nd"] = _dot(st["m"].astype(BF16), wide(PQ))

        def features(i):
            pk = _phi(paced(src[1][zr + e, _blk(i), :]))
            acc = st.get("z")
            for r in range(0, 128, 8):
                acc = pk[r:r + 8] if acc is None else acc + pk[r:r + 8]
            st["z"] = acc
            st["pk", i] = pk.astype(BF16)

        def update():
            lane_head = _iota((128, 128), 1) // DH
            upd = _dot(wide(VT), jnp.concatenate([st["pk", i] for i in range(4)], axis=0))
            z = jnp.sum(st["z"], axis=0, keepdims=True)
            m_old = st["m"]
            mem[g, :128, :] = m_old[:128] + jnp.where(_iota((128, 128), 0) // DH == lane_head, upd, 0.0)
            mem[g, 128:, :] = m_old[128:] + jnp.where(_iota((16, 128), 0) == lane_head[:16], z, 0.0)

        def qk(n, i, j):
            qt = abuf[e][QT][zr, i]
            zero = jnp.zeros((16, 128), I32)
            w = jnp.concatenate(
                [jnp.concatenate([qt[_blk(h, 16)] if hh == h else zero for hh in range(4)], axis=0)
                 for h in range(4)], axis=1)
            sc = _dot(_upk(abuf[e][KB][zr, j]), _upk(w))
            for h in range(4):
                blk = sc[:, _blk(h)]
                if j == i:
                    blk = blk + cmask[...]
                sbuf[e][i][zw, j, h] = blk
                acc = st.get(("mx", i, h))
                for r in range(0, 128, 8):
                    acc = blk[r:r + 8] if acc is None else jnp.maximum(acc, blk[r:r + 8])
                if j == i:
                    acc = jnp.broadcast_to(jnp.max(acc, axis=0, keepdims=True), (8, 128))
                st["mx", i, h] = acc

        def expo(n, i, j, h, r, nr):
            pr = jnp.exp2(sbuf[e][i][zr, j, h, r:r + nr, :] - jnp.tile(paced(st["mx", i, h]), (nr // 8, 1)))
            acc = st.get(("l", i, h))
            for k in range(0, nr, 8):
                acc = pr[k:k + 8] if acc is None else acc + pr[k:k + 8]
            st["l", i, h] = acc
            st.setdefault(("p", n, h), []).append(pr.astype(BF16))

        def pv(n, i, j):
            for h in range(4):
                a = _dot(_upk(abuf[e][VT][zr, j, _blk(h, 16), :]), jnp.concatenate(st.pop(("p", n, h)), axis=0))
                st["a", i, h] = a if j == 0 else st["a", i, h] + a

        def finish(i):
            outs = []
            for h in range(4):
                gh = gate[pl.ds(4 * g + h, 1), :]
                den = st["nd"][128 + h:129 + h, _blk(i)] + 1e-6
                num = st["nd"][_blk(h, DH), _blk(i)]
                lsum = jnp.sum(st["l", i, h], axis=0, keepdims=True)
                outs.append(num * (gh / den) + st["a", i, h] * ((1.0 - gh) / lsum))
            out = jnp.concatenate(outs, axis=0).T
            otmp[e][zw, _blk(i), :] = out
            pace["due"] = out[120:]

        c = CFG["a"]
        tasks = []
        for k, fn in enumerate((prepare_q, prepare_k, prepare_v)):
            tasks += _spread(max(t0 + c["prep"][k], ready[k]), c["prepd"], [lambda i=i, fn=fn: fn(i) for i in range(4)])
        tasks.append((t0 + c["ret"], retrieve))
        tasks.append((t0 + c["upd"], update))
        tasks += [(t0 + c["upd"] - c["featlag"] - (3 - i) * c["featd"], lambda i=i: features(i)) for i in range(4)]
        pieces = [(i, j) for i in c["units"] for j in range(i + 1)]
        tq = [c["qk0"] + n * c["qkd"] for n in range(10)]
        te = -1e9
        for n, (i, j) in enumerate(pieces):
            tasks.append((t0 + tq[n], lambda n=n, i=i, j=j: qk(n, i, j)))
            te = max(te + c["exd"], tq[n + i - j] + c["exlag"])
            tasks += _spread(t0 + te, c["exd"], [lambda n=n, i=i, j=j, h=h, r=r: expo(n, i, j, h, r, c["exr"])
                                                 for h in range(4) for r in range(0, 128, c["exr"])])
            tasks.append((t0 + te + c["pvlag"], lambda n=n, i=i, j=j: pv(n, i, j)))
            if j == i:
                tf = t0 + max(te + c["pvlag"], c["ret"]) + c["finlag"]
                tasks.append((tf, lambda i=i: finish(i)))
                if e == 1:
                    for k in range(2):
                        tasks.append((tf + c["putlag"] + k * c["putd"],
                                      lambda r=64 * i + 32 * k: put_o(p, r, 32, zr)))
        return tasks

    def attn_b(src, p, s, zr, zw, j):
        tasks = []
        c = CFG["b"]
        for e in range(2):
            tasks += attn_b_group(src, e, 2 * p + e, s, zr, zw, c["t0"][2 * j + e], ready(j))
        tasks += [(c["put0"][j] + r // 32 * c["putd"], lambda r=r: put_o(p, r, 32, zr)) for r in range(0, HL, 32)]
        return tasks

    def attn_b_group(src, e, g, s, zr, zw, t0, ready):
        st = {}

        def rnd(t):
            return lax.bitcast_convert_type(t.astype(BF16).astype(F32), I32)

        def pack(r, nr):
            if r == 0:
                kvn[e][zw, :HALO, :] = jnp.where(s > 0, halo[g], 0)
            sixteen = jnp.tile(paced(jnp.full((8, 128), 16, I32)), (nr // 8, 1))
            kv = rnd(src[1][zr + e, r:r + nr, :]) | lax.shift_right_logical(
                rnd(src[2][zr + e, r:r + nr, :]), sixteen)
            kvn[e][zw, HALO + r:HALO + r + nr, :] = kv
            if r + nr == L:
                halo[g] = kv[nr - HALO:]

        def flip(par, n):
            if n < 9:
                t = kvn[e][zr, pl.ds(HALO + par + 2 * n - 14, 128, stride=4), :]
            else:
                t = lax.bitcast_convert_type(src[0][zr + e, pl.ds(par + 2 * (n - 9), 128, stride=4), :], I32)
            kvt[e][par][zw, n] = flipped(t)

        def merge(x, y, sh):
            bit = (_iota((8, 128), 0) & sh) != 0
            return jnp.where(bit, y, x) + pltpu.roll(jnp.where(bit, x, y), sh, 0)

        def score(par, h, n):
            if n == 0:
                for a in range(2):
                    st["q", a] = lax.bitcast_convert_type(kvt[e][par][zr, 9 + a, _blk(h, DH), :], F32)
            high = jnp.tile(paced(jnp.full((8, 128), -65536, I32)), (4, 1))
            kk = lax.bitcast_convert_type(kvt[e][par][zr, n, _blk(h, DH), :] & high, F32)
            for a in range(2):
                w = 7 + a - n
                if 0 <= w < WIN:
                    t = st["q", a] * kk
                    t = (t[0:8] + t[8:16]) + (t[16:24] + t[24:32])
                    sh = 1
                    while sh < WIN and not w & sh:
                        t = merge(t, st.pop(("part", a, sh)), sh)
                        sh *= 2
                    st["part", a, sh] = t
                if w == 0:
                    sub = _iota((8, 128), 0)
                    valid = s * L + 4 * _iota((8, 128), 1) + (par + 2 * a) - DIL * sub >= 0
                    lg = jnp.where(valid, st.pop(("part", a, WIN)) * QSCALE, NEG)
                    pr = jnp.exp2(lg - jnp.max(lg, axis=0, keepdims=True))
                    st["p", par, h, a] = pr / jnp.sum(pr, axis=0, keepdims=True)

        def mix(par, h, n):
            sixteen = jnp.tile(paced(jnp.full((8, 128), 16, I32)), (4, 1))
            vv = lax.bitcast_convert_type(kvt[e][par][2 * zr, n, _blk(h, DH), :] << sixteen, F32)
            for a in range(2):
                w = 7 + a - n
                if 0 <= w < WIN:
                    t = st["p", par, h, a][w:w + 1] * vv
                    st["acc", a] = t if w == 7 else st["acc", a] + t
                if w == 0:
                    otr[e][par][zw, a, _blk(h, DH), :] = st["acc", a]

        def unflip(j):
            otmp[e][zw, pl.ds(j, 128, stride=4), :] = flipped(otr[e][j % 2][zr, j // 2])

        c = CFG["b"]
        tasks = _spread(max(t0 + c["pack0"], ready[2]), c["packd"], [lambda r=r: pack(r, 32) for r in range(0, L, 32)])
        hd = c["pard"] / 4
        for par in range(2):
            tasks += _spread(t0 + c["flip0"] + par * c["pard"], c["flipd"],
                             [lambda par=par, n=n: flip(par, n) for n in (9, 10, *range(9))])
            for h in range(4):
                t = t0 + c["sc0"] + par * c["pard"] + h * hd
                tasks += _spread(t, hd * c["scf"], [lambda par=par, h=h, n=n: score(par, h, n) for n in range(9)])
                t += hd * (c["scf"] + c["mixlag"])
                tasks += _spread(t, hd * (1 - c["scf"]),
                                 [lambda par=par, h=h, n=n: mix(par, h, n) for n in range(9)])
            for a in range(2):
                tasks.append((t + c["unlag"], lambda j=par + 2 * a: unflip(j)))
        return tasks

    def prepare_units(lo, hi):
        def body(u, carry):
            pltpu.make_async_copy(wraw.at[u], wraw.at[u], wsem.at[u]).wait()
            prep(u)
            return carry

        lax.fori_loop(lo, hi, body, 0)

    def widen(s):
        x_copy(s).wait()
        xres[s] = xio[s].astype(F32)

    def segment(n, carry):
        kind = (n // NSEG) % 2
        s = n % NSEG
        zr = lax.shift_right_logical(n, 8)
        zw = lax.shift_right_logical(n, 9)

        never[0] = zr > 0

        @pl.when(n == 0)
        def _():
            widen(n)
            start(range(3, 9))
            _weave((), norm(n, n, zr, 0, 1, 2), pace)
            prepare_units(0, 3)
            widen(n + 1)
            start(range(9, NUNIT))
            if CFG["only"] is None:
                _weave(proj(n, n, qkvs[0], zw), norm(n + 1, n + 1, zr, -1, 2.3, 1.5), pace)

        def steps(attn, nstep):
            def body(it, carry):
                if attn is attn_a:
                    first = jnp.minimum(3 + 3 * nstep * it, 12)
                    prepare_units(first, jnp.where(n == 0, jnp.minimum(first + 3 * nstep, 12), first))

                    @pl.when(jnp.logical_and(n == 0, it == 0))
                    def _():
                        x_copy(2).start()
                        x_copy(3).start()
                        start(range(NUNIT, 2 * NUNIT))

                per = 3 * 7 * HL // prow
                tasks, mains = [], []
                for j in range(nstep):
                    p = it * nstep + j
                    nn = n + (p + 1) // NPAIR
                    u0 = ((nn // NSEG) % 2) * NUNIT + ((p + 1) % NPAIR) * 3
                    tasks += [(t * per / 42, f) for t, f in attn(qkvs[j % 2], p, s, zr, zw, j)]
                    mains.append(proj(nn % 2, u0, qkvs[(j + 1) % 2], zw))
                _weave((m for g in mains for m in g), tasks, pace)
                return carry

            if nstep == NPAIR:
                body(0, 0)
            else:
                lax.fori_loop(0, NPAIR // nstep, body, 0)

        if CFG["only"] in (None, "a"):
            @pl.when(kind == 0)
            def _():
                with _scope("A"):
                    steps(attn_a, CFG["steps_a"])

        if CFG["only"] in (None, "b"):
            @pl.when(kind == 1)
            def _():
                with _scope("B"):
                    steps(attn_b, CFG["steps_b"])

        @pl.when(n < 2)
        def _():
            widen(n + 2)
            prepare_units(jnp.where(n == 0, 12, NUNIT), jnp.where(n == 0, NUNIT, 2 * NUNIT))

        if CFG["only"] in (None, "o"):
            with _scope("O"):
                c = CFG["o"]
                tasks = norm((n + 2) % NSEG, n % 2, zr, c["start"], c["step"], c["lag"])
                _weave(out_proj(kind * NUNIT + 12, s), tasks, pace)

        if CFG["only"] in ("a", "b"):
            xio[0, :16, :128] = os_[zr, zr, :16, :]
        if CFG["only"] == "o":
            xio[0, :16, :128] = _upk(xs[zr, zr, :8, :128])

        @pl.when(n >= 3 * NSEG)
        def _():
            pltpu.make_async_copy(
                xio.at[s], out_hbm.at[pl.ds(pl.multiple_of(s * L, L), L)], osem.at[s]).start()

        return carry

    lax.fori_loop(0, 4 * NSEG, segment, 0)
    for s in range(NSEG):
        pltpu.make_async_copy(xio.at[s], out_hbm.at[pl.ds(s * L, L)], osem.at[s]).wait()


CFG["a"] = dict(exr=128, t0=(3, 21.5, 40.5, 59), prep=(-6, -4, -2), prepd=2, ret=2, upd=12, units=(0, 1, 2, 3),
                qk0=0, qkd=1.4, exd=1.4, exlag=1.5, pvlag=2.8, finlag=1, putlag=2, putd=0.5, featlag=1.5, featd=0.5)
CFG["b"] = dict(t0=(-1, 17, 42, 58), pack0=0, packd=1, flip0=1, flipd=4, pard=8, sc0=6, scf=0.58,
                mixlag=0.3, unlag=1.5, put0=(43, 82), putd=0.25)
CFG["o"] = dict(start=-1, step=6, lag=3)


def build(interpret=False):
    any_spec = pl.BlockSpec(memory_space=pl.ANY)
    return pl.pallas_call(
        _kernel,
        out_shape=jax.ShapeDtypeStruct((S, D), BF16),
        in_specs=[any_spec] * 5 + [pl.BlockSpec(memory_space=pltpu.VMEM)] + [any_spec] * 2,
        out_specs=any_spec,
        scratch_shapes=[
            pltpu.VMEM((NSEG, L, D), BF16),
            pltpu.VMEM((NSEG, L, D), F32),
            pltpu.VMEM((1, L, D), F32),
            pltpu.VMEM((2, 7, HL // 2, D // 2), I32),
            pltpu.VMEM((NPAIR, 7, HL, 128), BF16),
            pltpu.VMEM((2 * NUNIT, D, 256), BF16),
            pltpu.VMEM((2 * NUNIT, 7, 256, 128), I32),
            *[pltpu.VMEM((2, L, 128), F32)] * 6,
            pltpu.VMEM((2 * NPAIR, 144, 128), F32),
            pltpu.VMEM((H, 128), F32),
            pltpu.VMEM((128, 128), F32),
            pltpu.VMEM((2 * NPAIR, HALO, 128), I32),
            pltpu.SemaphoreType.DMA((NSEG,)),
            pltpu.SemaphoreType.DMA((2 * NUNIT,)),
            pltpu.SemaphoreType.DMA((NSEG,)),
        ]
        + [pltpu.VMEM((1, HALO + L, 128), I32)] * 2
        + [pltpu.VMEM((1, L, 128), F32)] * 2
        + [pltpu.VMEM((1, 4, 64, 128), I32)] * 8
        + [pltpu.VMEM((1, i + 1, 4, 128, 128), F32) for i in range(4)] * 2
        + [pltpu.VMEM((1, 11, 128, 128), I32)] * 4
        + [pltpu.VMEM((1, 2, 128, 128), F32)] * 4,
        compiler_params=pltpu.CompilerParams(vmem_limit_bytes=110 * 2 ** 20, flags=CFG["flags"] or None),
        interpret=interpret,
        name="fused",
    )


@jax.jit
def pallas_interleave_layers__memory_aug_infini_attn__sliding_local_dilated__prompt_kernel(A_x, A_wq, A_wk, A_wv, A_wo, A_beta, B_x, B_wqkv, B_wo):
    del B_x
    out = build()(A_x.reshape(S, D), A_wq, A_wk, A_wv, A_wo, A_beta.reshape(1, H), B_wqkv, B_wo)
    return out.reshape(A_x.shape)
```

```python
import math

import jax
import jax.numpy as jnp
from jax import lax
import jax.experimental.pallas as pl
import jax.experimental.pallas.tpu as pltpu

S, D, H, DH = 2048, 1024, 32, 32
NSEG, L = 4, 512
HL = L // 2
NPAIR = 4
NUNIT = 16
STEP = 42
WIN, DIL = 8, 2
HALO = 16
PAD = 32
LOG2E = math.log2(math.e)
QSCALE = DH ** -0.5 * LOG2E
NEG = -1e9 * LOG2E
F32, BF16, I32 = jnp.float32, jnp.bfloat16, jnp.int32

PLAN_A = dict(
    start=(5, 22, 40.5, 58.5), q=(-6.3, -6.3, -6.6, -6.3), k=(-6, -3, -2.3, -3.3),
    v=(-1.4, -3.7, -2, -2.6), qkv_len=(2, 2, 1.7, 1.1), retrieve=(3.7, 4.3, 3.7, 1.7),
    update=(12.3, 13.3, 12.3, 12.3), feat_lead=(1.5, 3.1, 0.6, 0.9), feat_step=(0.6, 0.7, 0.8, 0.6),
    diag_len=(2.5,) * 4, qk_step=(2, 2.2, 1.95, 2.05), exp_step=(1.7, 1.7, 1.6, 1.5),
    exp_lag=(1.5, 0.5, 1.5, 1.2), pv_lag=(2.8, 2.5, 2.8, 2.8), finish_lag=(0, 1, 1, 1.6),
    put_lag=(0, 3, 0, 0.8), put_step=(0.95,) * 4)
PLAN_B = dict(
    start=(-1.6, 17.7, 41.4, 60.1, 83.4, 101.7, 125.4, 139.4), pack=(-0.2, -6, 0, -6, -0.3, -6, 0, -6),
    pack_len=(1, 2.3, 1, 3, 1, 2.6, 1, 3), flip0=(1, -2) * 4, flip1=(7, 6.4, 7, 6.4, 7, 6.4, 7, 7.6),
    flip_len=(4, 3.8, 4, 4, 4, 4, 4, 4), score=(6.5, 4, 6.5, 4, 6.5, 4, 8.5, 4),
    parity_len=(9, 9, 9, 9, 9.2, 9, 7.3, 8.4), score_part=(0.62,) * 8, unflip_lag=(1.2,) * 7 + (0.6,),
    put=(0, 44, 0, 86, 0, 128, 0, 163.5), put_step=(0, 0.2, 0, 0.32, 0, 0.2, 0, 0.2))


def _dot(a, b):
    return jnp.dot(a, b, preferred_element_type=F32)


def _iota(shape, axis):
    return lax.broadcasted_iota(I32, shape, axis)


def _words(x):
    return pltpu.bitcast(x.astype(BF16), I32)


def _halves(x):
    return pltpu.bitcast(x, BF16)


def _word_rows(start, size):
    return slice(start // 2, (start + size) // 2)


def _blk(i, n=128):
    return slice(i * n, (i + 1) * n)


def _token(half, r):
    return r // 64 * 128 + half * 64 + r % 64


def _phi(t):
    return jnp.where(t > 0, t + 1.0, jnp.exp(t))


def _lhs_terms(a11, a12, a21, a22):
    return (a11 + a22, a21 + a22, a11, a22, a11 + a12, a21 - a11, a12 - a22)


def _strassen(product, emit):
    m = product(0)
    c11 = c22 = m
    yield m
    m = product(6)
    c11 = c11 + m
    yield m
    m = product(5)
    c22 = c22 + m
    yield m
    c21 = product(3)
    c11 = c11 + c21
    yield c21
    m = product(1)
    c22 = c22 - m
    emit(1, 0, c21 + m)
    yield m
    c12 = product(4)
    emit(0, 0, c11 - c12)
    yield c12
    m = product(2)
    emit(1, 1, c22 + m)
    emit(0, 1, c12 + m)
    yield m


def _regroup(xs):
    lane = _iota(xs[3].shape, 1)

    def pick(bit, one, zero):
        if one is None and zero is None:
            return None
        return jnp.where((lane & bit) != 0, 0.0 if one is None else one, 0.0 if zero is None else zero)

    us = [pick(32, xs[(a + 1) % 4], xs[a]) for a in range(4)]
    return [pick(64, us[(2 - a) % 4], us[-a % 4]) for a in range(4)]


def _merge(op, x, y, sh):
    bit = (_iota((8, 128), 0) & sh) != 0
    return op(jnp.where(bit, y, x), pltpu.roll(jnp.where(bit, x, y), sh, 0))


def _reduce4(op, xs):
    t = _merge(op, _merge(op, xs[0], xs[1], 1), _merge(op, xs[2], xs[3], 1), 2)
    return op(t, pltpu.roll(t, 4, 0))


def _tree(op, xs):
    while len(xs) > 1:
        xs = [op(a, b) for a, b in zip(xs[0::2], xs[1::2])]
    return xs[0]


def _fold(op, acc, x):
    for r in range(0, x.shape[0], 8):
        acc = x[r:r + 8] if acc is None else op(acc, x[r:r + 8])
    return acc


def _spread(start, length, thunks):
    return [(start + length * k / len(thunks), f) for k, f in enumerate(thunks)]


class _Weaver:
    def __init__(self, never):
        self.never = never
        self.rows, self.count, self.waits = None, 0, {}

    def run(self, projections, tasks):
        tasks = sorted(tasks, key=lambda t: t[0])
        k = 0
        while k < len(tasks) and tasks[k][0] < 0:
            tasks[k][1]()
            k += 1
        for i, m in enumerate(m for products in projections for m in products):
            while k < len(tasks) and tasks[k][0] < i + 1:
                r = int((tasks[k][0] - i) * m.shape[0]) // 8 * 8
                self.rows = m[r:r + 8]
                tasks[k][1]()
                k += 1
        for _, thunk in tasks[k:]:
            thunk()
        self.rows, self.count, self.waits = None, 0, {}

    def paced(self, x):
        if self.rows is None:
            return x
        rows = lax.bitcast_convert_type(self.rows, x.dtype)
        return jnp.where(self.never, jnp.tile(rows, (x.shape[0] // 8, 1)), x)

    def transposed(self, x):
        return jnp.concatenate([self.paced(x[:8]), x[8:]], axis=0).T

    def constant(self, value, rows):
        return jnp.tile(self.paced(jnp.full((8, 128), value, I32)), (rows // 8, 1))

    def due(self, x):
        self.waits[self.count + 4] = x[-8:]

    def operand(self, w):
        head = w[:8]
        if self.count in self.waits:
            head = jnp.where(self.never, lax.bitcast_convert_type(self.waits.pop(self.count), I32), head)
        self.count += 1
        return jnp.concatenate([head, w[8:]], axis=0)


def _kernel(x_hbm, wq_hbm, wk_hbm, wv_hbm, woa_hbm, beta_ref, wqkv_hbm, wob_hbm, out_hbm,
            xio, xres, xtmp, xs, os_, wraw, wst, mem, gate, cmask, halo, xsem, wsem, osem, *bufs):
    bufs = list(bufs)
    kvn, otmp = ([bufs.pop(0) for _ in range(2)] for _ in range(2))
    qkv, abuf, sbuf, kvt, otr = (
        [[bufs.pop(0) for _ in range(k)] for _ in range(2)] for k in (3, 4, 4, 2, 2))

    def x0_copy(i):
        return pltpu.make_async_copy(x_hbm.at[_blk(i)], xio.at[0, _blk(i)], xsem.at[i])

    def x_copy(s):
        rows = pl.ds(pl.multiple_of(s * L, L), L)
        return pltpu.make_async_copy(x_hbm.at[rows], xio.at[s], xsem.at[s + 3])

    def w_copy(u):
        kind, v = divmod(u, NUNIT)
        if v >= 12:
            src, col = (woa_hbm, wob_hbm)[kind], (v - 12) * 256
        elif kind == 0:
            src, col = (wq_hbm, wk_hbm, wv_hbm)[v % 3], (v // 3) * 256
        else:
            src, col = wqkv_hbm, (v % 3) * D + (v // 3) * 256
        return pltpu.make_async_copy(src.at[:, pl.ds(col, 256)], wraw.at[u], wsem.at[u])

    def out_copy(s, i):
        rows = pl.ds(pl.multiple_of(s * L + i * 128, 128), 128)
        return pltpu.make_async_copy(xio.at[s, _blk(i)], out_hbm.at[rows], osem.at[4 * s + i])

    def fetch(lo, hi):
        for u in range(lo, hi):
            w_copy(u).start()

    for i in range(4):
        x0_copy(i).start()
    fetch(0, 1)

    row = _iota((64, H), 0)
    beta = jnp.broadcast_to(beta_ref[...].astype(F32), (64, H))
    beta = jnp.sum(jnp.where(row // 8 * 4 + row % 4 == _iota((64, H), 1), beta, 0.0), axis=1, keepdims=True)
    gate[...] = jnp.broadcast_to(1.0 / (1.0 + jnp.exp(-beta)), (64, 128)).reshape(8, 8, 128)
    cmask[...] = jnp.where(_iota((DH, 128), 0) <= _iota((DH, 128), 1) % DH, 0.0, NEG)

    def segment(n, carry):
        kind = (n // NSEG) % 2
        s = n % NSEG
        zr = lax.shift_right_logical(n, 8)
        zw = lax.shift_right_logical(n, 9)
        weaver = _Weaver(zr > 0)
        paced = weaver.paced

        def weight_terms(u):
            def rows(t, r):
                top = wraw[u, 256 * t + r:256 * t + r + 32, :]
                bot = wraw[u, 256 * t + 128 + r:256 * t + 128 + r + 32, :]
                b1, b2 = top.astype(F32), bot.astype(F32)
                b11, b12, b21, b22 = paced(b1[:, :128]), b1[:, 128:], b2[:, :128], paced(b2[:, 128:])
                terms = (b11 + b22, top[:, :128], b12 - b22, b21 - b11, bot[:, 128:], b11 + b12, b21 + b22)
                for i, term in enumerate(terms):
                    if term.dtype == BF16:
                        words = _words(term)
                    else:
                        words = _words(jnp.concatenate([term[:16], term[16:]], axis=1))
                        words = jnp.concatenate([words[:, :128], words[:, 128:]], axis=0)
                    wst[u, i, _word_rows(128 * t + r, 32), :] = words

            return [lambda t=t, r=r: rows(t, r) for t in range(4) for r in range(0, 128, 32)]

        def prepare_weights(lo, hi, fetch_more=False):
            def body(u, carry):
                pltpu.make_async_copy(wraw.at[u], wraw.at[u], wsem.at[u]).wait()
                if fetch_more:
                    pl.when(u == 6)(lambda: fetch(9, NUNIT))
                for thunk in weight_terms(u):
                    thunk()
                return carry

            lax.fori_loop(lo, hi, body, 0)

        def layernorm(sn, slot, start, step, lag, from_input=False):
            st = {}

            def mean(r):
                if from_input:
                    x = xio[sn, r:r + 16, :].astype(F32)
                    xres[sn, r:r + 16, :] = x
                else:
                    x = xres[sn, r:r + 16, :]
                xtmp[3 * zr, r:r + 16, :] = x
                acc = paced(x[:, :128])
                for t in range(1, 8):
                    acc = acc + x[:, _blk(t)]
                st["m", r] = jnp.broadcast_to(jnp.sum(acc, axis=1, keepdims=True) * (1.0 / D), (16, 128))

            def scale(r):
                m = paced(st["m", r])
                acc = None
                for t in range(8):
                    c = xtmp[zr, r:r + 16, _blk(t)] - m
                    acc = c * c if acc is None else acc + c * c
                var = jnp.sum(acc, axis=1, keepdims=True) * (1.0 / D)
                st["r", r] = jnp.broadcast_to(lax.rsqrt(var + 1e-5), (16, 128))

            def terms(r, t):
                ys = []
                for r0 in (_token(0, r), _token(1, r)):
                    m = paced(st["m", r0])
                    ys += [(xtmp[2 * zr, r0:r0 + 16, _blk(2 * t + k)] - m) * st["r", r0] for k in range(2)]
                for i, term in enumerate(_lhs_terms(*ys)):
                    words = _words(term)
                    xs[slot, i, _word_rows(r, 16), _blk(t)] = words
                weaver.due(words)

            tasks = []
            for k, r in enumerate(range(0, HL, 16)):
                t0 = start + k * step
                rows = (_token(0, r), _token(1, r))
                tasks += _spread(t0, step, [lambda r0=r0: mean(r0) for r0 in rows])
                tasks += _spread(t0 + lag, step, [lambda r0=r0: scale(r0) for r0 in rows])
                tasks += _spread(t0 + 2 * lag + step / 2, step, [lambda r=r, t=t: terms(r, t) for t in range(4)])
            return tasks

        def project_in(slot, u0, dst):
            for c in range(3):
                for r in range(0, HL, 128):
                    def product(i):
                        lhs = _halves(xs[slot, i, _word_rows(r, 128), :])
                        return _dot(lhs, _halves(weaver.operand(wst[u0 + c, i])))

                    def emit(bi, bj, val):
                        for k in (0, 64):
                            dst[c][zw + bj, pl.ds(_token(bi, r + k), 64), :] = val[k:k + 64]

                    yield from _strassen(product, emit)

        def project_out(u0, stage_output):
            for r in range(0, HL, 64):
                for v in range(4):
                    def product(i):
                        lhs = jnp.concatenate([os_[t, i, r:r + 64, :] for t in range(NPAIR)], axis=1)
                        return _dot(lhs, _halves(weaver.operand(wst[u0 + v, i])))

                    def emit(bi, bj, val):
                        rows = pl.ds(_token(bi, r), 64)
                        y = xres[s, rows, _blk(2 * v + bj)] + val
                        xres[s, rows, _blk(2 * v + bj)] = y
                        if stage_output:
                            xio[s, rows, _blk(2 * v + bj)] = y.astype(BF16)

                    yield from _strassen(product, emit)

        def put_heads(p, r):
            top, bot = pl.ds(_token(0, r), 32), pl.ds(_token(1, r), 32)
            terms = _lhs_terms(paced(otmp[0][zr, top]), otmp[1][zr, top],
                               otmp[0][zr, bot], paced(otmp[1][zr, bot]))
            for i, term in enumerate(terms):
                os_[p + zr, i, r:r + 32, :] = term.astype(BF16)

        def attention_a(src, p, e, plan, ready):
            g = 2 * p + e
            kb, vt, qt, fq = abuf[e]
            st = {}

            def prepare_q(i):
                q = weaver.transposed(src[0][zr + e, _blk(i), :])
                turned = [pltpu.roll(q[_blk(h, DH)], DH * h, 1) if h else q[:DH] for h in range(4)]
                qt[zw, i] = _words(jnp.concatenate(turned, axis=0) * QSCALE)
                fq[zw, i] = _words(_phi(q))

            def prepare_k(i):
                kb[zw, i] = _words(paced(src[1][zr + e, _blk(i), :]))

            def prepare_v(i):
                vt[zw, i] = _words(weaver.transposed(src[2][zr + e, _blk(i), :]))

            def whole(buf):
                return _halves(jnp.concatenate([buf[zr, i] for i in range(4)], axis=1))

            def retrieve():
                st["m"] = jnp.where(s > 0, mem[g], 0.0)
                st["nd"] = _dot(st["m"].astype(BF16), whole(fq))

            def features(i):
                fk = _phi(paced(src[1][zr + e, _blk(i), :]))
                st["z"] = _fold(jnp.add, st.get("z"), fk)
                st["fk", i] = fk.astype(BF16)

            def update():
                head = _iota((128, 128), 1) // DH
                upd = _dot(whole(vt), jnp.concatenate([st["fk", i] for i in range(4)], axis=0))
                z = jnp.sum(st["z"], axis=0, keepdims=True)
                mem[g, :128, :] = st["m"][:128] + jnp.where(_iota((128, 128), 0) // DH == head, upd, 0.0)
                mem[g, 128:, :] = st["m"][128:] + jnp.where(_iota((16, 128), 0) == head[:16], z, 0.0)

            def close_max(i):
                mx = _reduce4(jnp.maximum, [st["mx", i, h] for h in range(4)])
                for h in range(4):
                    st["mx", i, h] = jnp.broadcast_to(mx[h:h + 1], (8, 128))
                for c, mx in enumerate(_regroup([st["mx", i, h] for h in range(4)])):
                    st["dmx", i, c] = mx

            def qk_diagonal(c):
                keep = (_iota((64, 128), 1) // DH - _iota((64, 128), 0) // 16) % 4 == c
                nk = DH * (c + 1)
                for i in range(4):
                    sc = _dot(_halves(kb[zr, i, :nk // 2, :]), _halves(jnp.where(keep, qt[zr, i], 0)))
                    last = sc[nk - DH:] + cmask[...]
                    sc = jnp.concatenate([sc[:nk - DH], last], axis=0) if c else last
                    sbuf[e][0][zw, i, c, :nk, :] = sc
                    st["dmx", i, c] = _fold(jnp.maximum, None, sc)

            def open_max():
                for i in range(4):
                    for h, mx in enumerate(_regroup([st["dmx", i, c] for c in range(4)])):
                        st["mx", i, h] = mx
                close_max(0)

            def qk(i, j):
                q = qt[zr, i]
                zero = jnp.zeros((16, 128), I32)
                w = jnp.concatenate(
                    [jnp.concatenate([q[_blk(h, 16)] if hh == h else zero for hh in range(4)], axis=0)
                     for h in range(4)], axis=1)
                sc = _dot(_halves(kb[zr, j]), _halves(w))
                for h in range(4):
                    sbuf[e][i][zw, j, h] = sc[:, _blk(h)]
                    st["mx", i, h] = _fold(jnp.maximum, st["mx", i, h], sc[:, _blk(h)])
                if j == i - 1:
                    close_max(i)

            def exponentiate(i, j, k):
                if j < i:
                    pr = jnp.exp2(sbuf[e][i][zr, j, k] - jnp.tile(paced(st["mx", i, k]), (16, 1)))
                    st["l", i, k] = _fold(jnp.add, st.get(("l", i, k)), pr)
                    st["p", i, j, k] = [pr.astype(BF16)]
                    return
                prs = [None] * 4
                for c in range(k, 4):
                    sc = sbuf[e][0][zr, i, c, _blk(k, DH), :]
                    prs[c] = jnp.exp2(sc - jnp.tile(paced(st["dmx", i, c]), (4, 1)))
                    st["dl", i, c] = _fold(jnp.add, st.get(("dl", i, c)), prs[c])
                for h, pr in enumerate(_regroup(prs)):
                    st.setdefault(("p", i, j, h), []).append(pr.astype(BF16))

            def pv(i, j):
                for h in range(4):
                    pr = jnp.concatenate(st.pop(("p", i, j, h)), axis=0)
                    a = _dot(_halves(vt[zr, j, _blk(h, 16), :]), pr)
                    st["a", i, h] = a if j == 0 else st["a", i, h] + a

            def finish(i):
                sums = _regroup([st["dl", i, c] for c in range(4)])
                sums = _reduce4(jnp.add, [x + st["l", i, h] if i else x for h, x in enumerate(sums)])
                local = (1.0 - gate[g]) / sums
                memory = gate[g] / (st["nd"][128:136, _blk(i)] + 1e-6)
                outs = []
                for h in range(4):
                    a = st["a", i, h] * local[h:h + 1]
                    outs.append(st["nd"][_blk(h, DH), _blk(i)] * memory[h:h + 1]
                                + (pltpu.roll(a, 128 - DH * h, 1) if h else a))
                out = jnp.concatenate(outs, axis=0).T
                otmp[e][zw, _blk(i), :] = out
                weaver.due(out)

            t0 = plan["start"]
            tasks = []
            for c, fn in enumerate((prepare_q, prepare_k, prepare_v)):
                tasks += _spread(max(t0 + plan["qkv"[c]], ready[c]), plan["qkv_len"],
                                 [lambda i=i, fn=fn: fn(i) for i in range(4)])
            tasks.append((t0 + plan["retrieve"], retrieve))
            tasks.append((t0 + plan["update"], update))
            tasks += [(t0 + plan["update"] - plan["feat_lead"] - (3 - i) * plan["feat_step"],
                       lambda i=i: features(i)) for i in range(4)]
            tasks += _spread(t0, plan["diag_len"], [lambda c=c: qk_diagonal(c) for c in (3, 2, 1, 0)] + [open_max])
            tq = t0 + plan["diag_len"]
            closed = {0: tq}
            for i in range(4):
                for j in range(i):
                    tasks.append((tq, lambda i=i, j=j: qk(i, j)))
                    closed[i] = tq
                    tq += plan["qk_step"]
            te = -math.inf
            for i in range(4):
                for j in range(i + 1):
                    te = max(te + plan["exp_step"], closed[i] + plan["exp_lag"])
                    tasks += _spread(te, plan["exp_step"],
                                     [lambda i=i, j=j, k=k: exponentiate(i, j, k) for k in range(4)])
                    tasks.append((te + plan["pv_lag"], lambda i=i, j=j: pv(i, j)))
                tf = max(te + plan["pv_lag"], t0 + plan["retrieve"]) + plan["finish_lag"]
                tasks.append((tf, lambda i=i: finish(i)))
                if e == 1:
                    tasks += [(tf + plan["put_lag"] + k * plan["put_step"],
                               lambda r=64 * i + 32 * k: put_heads(p, r)) for k in range(2)]
            return tasks

        def attention_b(src, p, e, plan, ready):
            g = 2 * p + e
            st = {}

            def bits(t):
                return lax.bitcast_convert_type(t.astype(BF16).astype(F32), I32)

            def pack(r):
                if r == 0:
                    kvn[e][zw, :HALO, :] = jnp.where(s > 0, halo[g], 0)
                sixteen = weaver.constant(16, 32)
                kv = bits(src[1][zr + e, r:r + 32, :]) | lax.shift_right_logical(
                    bits(src[2][zr + e, r:r + 32, :]), sixteen)
                kvn[e][zw, HALO + r:HALO + r + 32, :] = kv
                if r + 32 == L:
                    halo[g] = kv[32 - HALO:]

            def flip(par, t):
                if t < 9:
                    x = kvn[e][zr, pl.ds(HALO + par + 2 * t - 14, 128, stride=4), :]
                else:
                    x = lax.bitcast_convert_type(src[0][zr + e, pl.ds(par + 2 * (t - 9), 128, stride=4), :], I32)
                kvt[e][par][zw, t] = weaver.transposed(x)

            def score(par, h, t):
                high = weaver.constant(-65536, DH)
                k = lax.bitcast_convert_type(kvt[e][par][zr, t, _blk(h, DH), :] & high, F32)
                for a in range(2):
                    w = 7 + a - t
                    if 0 <= w < WIN:
                        x = lax.bitcast_convert_type(kvt[e][par][(3 + t) * zr, 9 + a, _blk(h, DH), :], F32) * k
                        x = (x[0:8] + x[8:16]) + (x[16:24] + x[24:32])
                        sh = 1
                        while (4 * a + h) & sh:
                            x = _merge(jnp.add, st.pop(("part", par, w, sh)), x, sh)
                            sh *= 2
                        st["part", par, w, sh] = x

            def softmax(par):
                token = s * L + 4 * _iota((8, 128), 1) + par + 2 * (_iota((8, 128), 0) // 4)
                lg = [paced(st.pop(("part", par, w, 8))) * QSCALE for w in range(WIN)]
                lg = [jnp.where(token >= DIL * w, x, NEG) for w, x in enumerate(lg)]
                mx = _tree(jnp.maximum, lg)
                pr = [jnp.exp2(x - mx) for x in lg]
                inv = 1.0 / _tree(jnp.add, pr)
                st["p", par] = [x * inv for x in pr]

            def mix(par, h, t):
                sixteen = weaver.constant(16, DH)
                v = lax.bitcast_convert_type(kvt[e][par][2 * zr, t, _blk(h, DH), :] << sixteen, F32)
                for a in range(2):
                    w = 7 + a - t
                    if 0 <= w < WIN:
                        x = st["p", par][w][4 * a + h:4 * a + h + 1] * v
                        st["acc", par, a] = x if w == WIN - 1 else st["acc", par, a] + x
                    if w == 0:
                        otr[e][par][zw, a, _blk(h, DH), :] = st["acc", par, a]

            def unflip(par, a):
                otmp[e][zw, pl.ds(par + 2 * a, 128, stride=4), :] = weaver.transposed(otr[e][par][zr, a])

            t0 = plan["start"]
            tasks = _spread(max(t0 + plan["pack"], ready[2]), plan["pack_len"],
                            [lambda r=r: pack(r) for r in range(0, L, 32)])
            score_len = plan["parity_len"] * plan["score_part"]
            mix_len = plan["parity_len"] * (1 - plan["score_part"])
            for par in range(2):
                tasks += _spread(t0 + plan["flip%d" % par], plan["flip_len"],
                                 [lambda par=par, t=t: flip(par, t) for t in (9, 10, *range(9))])
                tp = t0 + plan["score"] + par * plan["parity_len"]
                tasks += _spread(tp, score_len, [lambda par=par, h=h, t=t: score(par, h, t)
                                                 for t in range(9) for h in range(4)])
                tp = tp + score_len + 0.5
                tasks.append((tp, lambda par=par: softmax(par)))
                tasks += _spread(tp + 0.5, mix_len, [lambda par=par, h=h, t=t: mix(par, h, t)
                                                     for h in range(4) for t in range(9)])
                tp += 0.5 + mix_len
                tasks += [(tp + plan["unflip_lag"], lambda par=par, a=a: unflip(par, a)) for a in range(2)]
            if e == 1:
                tasks += [(plan["put"] + k * plan["put_step"], lambda r=32 * k: put_heads(p, r)) for k in range(8)]
            return tasks

        def pairs(attention, plans, first, count):
            projections, tasks = [], []
            for j in range(count):
                p = first + j
                nxt = n + (p + 1) // NPAIR
                u0 = ((nxt // NSEG) % 2) * NUNIT + ((p + 1) % NPAIR) * 3
                ready = [STEP * (j - 1) + STEP // 3 * (c + 1) - 0.01 if j else -1 for c in range(3)]
                for e in range(2):
                    plan = {name: column[2 * j + e] for name, column in plans.items()}
                    tasks += attention(qkv[j % 2], p, e, plan, ready)
                projections.append(project_in(nxt % 2, u0, qkv[(j + 1) % 2]))
            return projections, tasks

        @pl.when(n == 0)
        def _():
            def arrive(i):
                x0_copy(i).wait()
                if i == 1:
                    x_copy(1).start()
                else:
                    fetch(*{0: (1, 3), 2: (3, 6), 3: (6, 9)}[i])

            weaver.run((), [(4 * i - 0.5, lambda i=i: arrive(i)) for i in range(4)]
                       + layernorm(0, 0, 0, 1, 1, from_input=True))
            prepare_weights(0, 1)
            tasks = [(12, x_copy(1).wait)] + layernorm(1, 1, 12, 25 / 16, 1.5, from_input=True)
            for u, t in ((1, 2), (2, 7)):
                tasks += [(t, w_copy(u).wait)] + _spread(t, 5, weight_terms(u))
            weaver.run([project_in(0, 0, qkv[0])], tasks)

        @pl.when(kind == 0)
        def _():
            def half(it, carry):
                @pl.when(jnp.logical_and(n == 0, it == 1))
                def _():
                    x_copy(2).start()
                    x_copy(3).start()
                    fetch(NUNIT, 2 * NUNIT)

                lo = 3 + 6 * it
                prepare_weights(lo, jnp.where(n == 0, 9 + 3 * it, lo), fetch_more=True)
                weaver.run(*pairs(attention_a, PLAN_A, 2 * it, 2))
                return carry

            lax.fori_loop(0, 2, half, 0)

            @pl.when(n < 2)
            def _():
                x_copy(n + 2).wait()
                xres[n + 2] = xio[n + 2].astype(F32)
                prepare_weights(jnp.where(n == 0, 12, NUNIT), jnp.where(n == 0, NUNIT, 2 * NUNIT))

            weaver.run([project_out(12, False)], layernorm((n + 2) % NSEG, n % 2, -1, 6, 3))

        @pl.when(kind == 1)
        def _():
            def send(i):
                pl.when(n >= 3 * NSEG)(lambda: out_copy(s, i).start())

            projections, tasks = pairs(attention_b, PLAN_B, 0, NPAIR)
            tasks += layernorm((n + 2) % NSEG, n % 2, STEP * NPAIR, 6, 3)
            tasks += [(STEP * NPAIR + 28 * (i + 1) + 3, lambda i=i: send(i)) for i in range(4)]
            weaver.run(projections + [project_out(NUNIT + 12, True)], tasks)

        return carry

    lax.fori_loop(0, 4 * NSEG, segment, 0)
    for s in range(NSEG):
        for i in range(4):
            out_copy(s, i).wait()


def _call(**kwargs):
    hbm = pl.BlockSpec(memory_space=pl.ANY)
    return pl.pallas_call(
        _kernel,
        out_shape=jax.ShapeDtypeStruct((S, D), BF16),
        in_specs=[hbm] * 5 + [pl.BlockSpec(memory_space=pltpu.VMEM)] + [hbm] * 2,
        out_specs=hbm,
        scratch_shapes=[
            pltpu.VMEM((NSEG, L, D), BF16),
            pltpu.VMEM((NSEG, L, D), F32),
            pltpu.VMEM((1, L, D), F32),
            pltpu.VMEM((2, 7, HL // 2, D // 2), I32),
            pltpu.VMEM((NPAIR, 7, HL, 128), BF16),
            pltpu.VMEM((2 * NUNIT, D, 256), BF16),
            pltpu.VMEM((2 * NUNIT, 7, 256, 128), I32),
            pltpu.VMEM((2 * NPAIR, 144, 128), F32),
            pltpu.VMEM((2 * NPAIR, 8, 128), F32),
            pltpu.VMEM((DH, 128), F32),
            pltpu.VMEM((2 * NPAIR, HALO, 128), I32),
            pltpu.SemaphoreType.DMA((NSEG + 3,)),
            pltpu.SemaphoreType.DMA((2 * NUNIT,)),
            pltpu.SemaphoreType.DMA((4 * NSEG,)),
        ]
        + [pltpu.VMEM((1, HALO + L + PAD, 128), I32)] * 2
        + [pltpu.VMEM((1, L + PAD, 128), F32)] * 2
        + [pltpu.VMEM((2, L + PAD, 128), F32)] * 6
        + [pltpu.VMEM((1, 4, 64, 128), I32)] * 8
        + [pltpu.VMEM((1, i or 4, 4, 128, 128), F32) for i in range(4)] * 2
        + [pltpu.VMEM((1, 11, 128, 128), I32)] * 4
        + [pltpu.VMEM((1, 2, 128, 128), F32)] * 4,
        compiler_params=pltpu.CompilerParams(vmem_limit_bytes=110 * 2 ** 20),
        name="fused",
        **kwargs,
    )


@jax.jit
def pallas_interleave_layers__memory_aug_infini_attn__sliding_local_dilated__prompt_kernel(
    A_x: jax.Array,
    A_wq: jax.Array,
    A_wk: jax.Array,
    A_wv: jax.Array,
    A_wo: jax.Array,
    A_beta: jax.Array,
    B_x: jax.Array,
    B_wqkv: jax.Array,
    B_wo: jax.Array,
):
    del B_x
    out = _call()(A_x.reshape(S, D), A_wq, A_wk, A_wv, A_wo, A_beta.reshape(1, H), B_wqkv, B_wo)
    return out.reshape(A_x.shape)
```

```python
import math

import jax
import jax.numpy as jnp
from jax import lax
import jax.experimental.pallas as pl
import jax.experimental.pallas.tpu as pltpu

S, D, H, DH = 2048, 1024, 32, 32
NSEG, L = 4, 512
HL = L // 2
NPAIR = 4
NUNIT = 16
STEP = 42
WIN, DIL = 8, 2
HALO = 16
PAD = 32
LOG2E = math.log2(math.e)
QSCALE = DH ** -0.5 * LOG2E
NEG = -1e9 * LOG2E
F32, BF16, I32 = jnp.float32, jnp.bfloat16, jnp.int32

PLAN_A = dict(
    start=(5, 22, 40.5, 58.5), q=(-6.3, -6.3, -6.6, -6.3), k=(-6, -3, -2.3, -3.3),
    v=(-1.4, -3.7, -2, -2.6), qkv_len=(2, 2, 1.7, 1.1), retrieve=(3.7, 4.3, 3.7, 1.7),
    update=(12.3, 13.3, 12.3, 12.3), feat_lead=(1.5, 3.1, 0.6, 0.9), feat_step=(0.6, 0.7, 0.8, 0.6),
    diag_len=(2.5,) * 4, qk_step=(2, 2.2, 1.95, 2.05), exp_step=(1.7, 1.7, 1.6, 1.5),
    exp_lag=(1.5, 0.5, 1.5, 1.2), pv_lag=(2.8, 2.5, 2.8, 2.8), finish_lag=(0, 1, 1, 1.6),
    put_lag=(0, 3, 0, 0.8), put_step=(0.95,) * 4)
PLAN_B = dict(
    start=(-1.6, 17.7, 41.4, 60.1, 83.4, 101.7, 125.4, 139.4), pack=(-0.2, -6, 0, -6, -0.3, -6, 0, -6),
    pack_len=(1, 2.3, 1, 3, 1, 2.6, 1, 3), flip0=(1, -2) * 4, flip1=(7, 6.4, 7, 6.4, 7, 6.4, 7, 7.6),
    flip_len=(4, 3.8, 4, 4, 4, 4, 4, 4), score=(6.5, 4, 6.5, 4, 6.5, 4, 8.5, 4),
    parity_len=(9, 9, 9, 9, 9.2, 9, 7.3, 8.4), score_part=(0.62,) * 8, unflip_lag=(1.2,) * 7 + (0.6,),
    put=(0, 44, 0, 86, 0, 128, 0, 162.9), put_step=(0, 0.2, 0, 0.32, 0, 0.2, 0, 0.2))


def _dot(a, b):
    return jnp.dot(a, b, preferred_element_type=F32)


def _iota(shape, axis):
    return lax.broadcasted_iota(I32, shape, axis)


def _words(x):
    return pltpu.bitcast(x.astype(BF16), I32)


def _halves(x):
    return pltpu.bitcast(x, BF16)


def _word_rows(start, size):
    return slice(start // 2, (start + size) // 2)


def _blk(i, n=128):
    return slice(i * n, (i + 1) * n)


def _token(half, r):
    return r // 64 * 128 + half * 64 + r % 64


def _phi(t):
    return jnp.where(t > 0, t + 1.0, jnp.exp(t))


def _lhs_terms(a11, a12, a21, a22):
    return (a11 + a22, a21 + a22, a11, a22, a11 + a12, a21 - a11, a12 - a22)


def _strassen(product, emit):
    m = product(0)
    c11 = c22 = m
    yield m
    m = product(6)
    c11 = c11 + m
    yield m
    m = product(5)
    c22 = c22 + m
    yield m
    c21 = product(3)
    c11 = c11 + c21
    yield c21
    m = product(1)
    c22 = c22 - m
    emit(1, 0, c21 + m)
    yield m
    c12 = product(4)
    emit(0, 0, c11 - c12)
    yield c12
    m = product(2)
    emit(1, 1, c22 + m)
    emit(0, 1, c12 + m)
    yield m


def _regroup(xs):
    lane = _iota(xs[3].shape, 1)

    def pick(bit, one, zero):
        if one is None and zero is None:
            return None
        return jnp.where((lane & bit) != 0, 0.0 if one is None else one, 0.0 if zero is None else zero)

    us = [pick(32, xs[(a + 1) % 4], xs[a]) for a in range(4)]
    return [pick(64, us[(2 - a) % 4], us[-a % 4]) for a in range(4)]


def _merge(op, x, y, sh):
    bit = (_iota((8, 128), 0) & sh) != 0
    return op(jnp.where(bit, y, x), pltpu.roll(jnp.where(bit, x, y), sh, 0))


def _reduce4(op, xs):
    t = _merge(op, _merge(op, xs[0], xs[1], 1), _merge(op, xs[2], xs[3], 1), 2)
    return op(t, pltpu.roll(t, 4, 0))


def _tree(op, xs):
    while len(xs) > 1:
        xs = [op(a, b) for a, b in zip(xs[0::2], xs[1::2])]
    return xs[0]


def _fold(op, acc, x):
    for r in range(0, x.shape[0], 8):
        acc = x[r:r + 8] if acc is None else op(acc, x[r:r + 8])
    return acc


def _spread(start, length, thunks):
    return [(start + length * k / len(thunks), f) for k, f in enumerate(thunks)]


class _Weaver:
    def __init__(self, never):
        self.never = never
        self.rows, self.count, self.waits = None, 0, {}

    def run(self, projections, tasks):
        tasks = sorted(tasks, key=lambda t: t[0])
        k = 0
        while k < len(tasks) and tasks[k][0] < 0:
            tasks[k][1]()
            k += 1
        for i, m in enumerate(m for products in projections for m in products):
            while k < len(tasks) and tasks[k][0] < i + 1:
                r = int((tasks[k][0] - i) * m.shape[0]) // 8 * 8
                self.rows = m[r:r + 8]
                tasks[k][1]()
                k += 1
        for _, thunk in tasks[k:]:
            thunk()
        self.rows, self.count, self.waits = None, 0, {}

    def paced(self, x):
        if self.rows is None:
            return x
        rows = lax.bitcast_convert_type(self.rows, x.dtype)
        return jnp.where(self.never, jnp.tile(rows, (x.shape[0] // 8, 1)), x)

    def transposed(self, x):
        return jnp.concatenate([self.paced(x[:8]), x[8:]], axis=0).T

    def constant(self, value, rows):
        return jnp.tile(self.paced(jnp.full((8, 128), value, I32)), (rows // 8, 1))

    def due(self, x):
        self.waits[self.count + 4] = x[-8:]

    def operand(self, w):
        head = w[:8]
        if self.count in self.waits:
            head = jnp.where(self.never, lax.bitcast_convert_type(self.waits.pop(self.count), I32), head)
        self.count += 1
        return jnp.concatenate([head, w[8:]], axis=0)


def _kernel(x_hbm, wq_hbm, wk_hbm, wv_hbm, woa_hbm, beta_hbm, wqkv_hbm, wob_hbm, out_hbm,
            xio, xres, xtmp, xs, os_, wraw, wst, wsa, mem, gate, cmask, halo, xsem, wsem, osem, bsem, *bufs):
    *bufs, beta_ref = bufs
    kvn, otmp = ([bufs.pop(0) for _ in range(2)] for _ in range(2))
    qkv, abuf, sbuf, kvt, otr = (
        [[bufs.pop(0) for _ in range(k)] for _ in range(2)] for k in (3, 4, 4, 2, 2))

    def x0_copy(i):
        return pltpu.make_async_copy(x_hbm.at[_blk(i)], xio.at[0, _blk(i)], xsem.at[i])

    def x_copy(s):
        rows = pl.ds(pl.multiple_of(s * L, L), L)
        return pltpu.make_async_copy(x_hbm.at[rows], xio.at[s], xsem.at[s + 3])

    def w_copy(u):
        kind, v = divmod(u, NUNIT)
        if v >= 12:
            src, col = (woa_hbm, wob_hbm)[kind], (v - 12) * 256
        elif kind == 0:
            src, col = (wq_hbm, wk_hbm, wv_hbm)[v % 3], (v // 3) * 256
        else:
            src, col = wqkv_hbm, (v % 3) * D + (v // 3) * 256
        return pltpu.make_async_copy(src.at[:, pl.ds(col, 256)], wraw.at[u], wsem.at[u])

    def out_copy(s, i):
        rows = pl.ds(pl.multiple_of(s * L + i * 128, 128), 128)
        return pltpu.make_async_copy(xio.at[s, _blk(i)], out_hbm.at[rows], osem.at[4 * s + i])

    def fetch(lo, hi):
        for u in range(lo, hi):
            w_copy(u).start()

    beta_copy = pltpu.make_async_copy(beta_hbm, beta_ref, bsem)
    beta_copy.start()
    for i in range(4):
        x0_copy(i).start()
    fetch(0, 1)
    beta_copy.wait()

    row = _iota((64, H), 0)
    beta = jnp.broadcast_to(beta_ref[...].astype(F32), (64, H))
    beta = jnp.sum(jnp.where(row // 8 * 4 + row % 4 == _iota((64, H), 1), beta, 0.0), axis=1, keepdims=True)
    gate[...] = jnp.broadcast_to(1.0 / (1.0 + jnp.exp(-beta)), (64, 128)).reshape(8, 8, 128)
    cmask[...] = jnp.where(_iota((DH, 128), 0) <= _iota((DH, 128), 1) % DH, 0.0, NEG)

    def segment(n, carry):
        kind = (n // NSEG) % 2
        s = n % NSEG
        zr = lax.shift_right_logical(n, 8)
        zw = lax.shift_right_logical(n, 9)
        weaver = _Weaver(zr > 0)
        paced = weaver.paced

        def weight_terms(u, dst=wst, first=0):
            def rows(t, r):
                top = wraw[u, 256 * t + r:256 * t + r + 16, :]
                bot = wraw[u, 256 * t + 128 + r:256 * t + 128 + r + 16, :]
                b1, b2 = top.astype(F32), bot.astype(F32)
                b11, b12, b21, b22 = paced(b1[:, :128]), b1[:, 128:], b2[:, :128], paced(b2[:, 128:])
                sums = _words(jnp.concatenate((b11 + b22, b12 - b22, b21 - b11, b11 + b12, b21 + b22), axis=1))
                sums = [sums[:, _blk(i)] for i in range(5)]
                terms = (sums[0], paced(_words(top[:, :128])), sums[1], sums[2], paced(_words(bot[:, 128:])),
                         sums[3], sums[4])
                for i, term in enumerate(terms):
                    dst[u - first, i, _word_rows(128 * t + r, 16), :] = term

            return [lambda t=t, r=r: rows(t, r) for t in range(4) for r in range(0, 128, 16)]

        def prepare_weights(lo, hi, also=lambda u: None, *where):
            def body(u, carry):
                pltpu.make_async_copy(wraw.at[u], wraw.at[u], wsem.at[u]).wait()
                also(u)
                for thunk in weight_terms(u, *where):
                    thunk()
                return carry

            lax.fori_loop(lo, hi, body, 0)

        def layernorm(sn, slot, start, step, lag, from_input=False):
            st = {}

            def mean(r):
                if from_input:
                    x = xio[sn, r:r + 16, :].astype(F32)
                    xres[sn, r:r + 16, :] = x
                else:
                    x = xres[sn, r:r + 16, :]
                xtmp[3 * zr, r:r + 16, :] = x
                acc = paced(x[:, :128])
                for t in range(1, 8):
                    acc = acc + x[:, _blk(t)]
                st["m", r] = jnp.broadcast_to(jnp.sum(acc, axis=1, keepdims=True) * (1.0 / D), (16, 128))

            def scale(r):
                m = paced(st["m", r])
                acc = None
                for t in range(8):
                    c = xtmp[zr, r:r + 16, _blk(t)] - m
                    acc = c * c if acc is None else acc + c * c
                var = jnp.sum(acc, axis=1, keepdims=True) * (1.0 / D)
                st["r", r] = jnp.broadcast_to(lax.rsqrt(var + 1e-5), (16, 128))

            def terms(r, t):
                ys = []
                for r0 in (_token(0, r), _token(1, r)):
                    m = paced(st["m", r0])
                    ys += [(xtmp[2 * zr, r0:r0 + 16, _blk(2 * t + k)] - m) * st["r", r0] for k in range(2)]
                words = _words(jnp.concatenate(_lhs_terms(*ys), axis=1))
                for i in range(7):
                    xs[slot, i, _word_rows(r, 16), _blk(t)] = words[:, _blk(i)]
                weaver.due(words[:, _blk(6)])

            tasks = []
            for k, r in enumerate(range(0, HL, 16)):
                t0 = start + k * step
                rows = (_token(0, r), _token(1, r))
                tasks += _spread(t0, step, [lambda r0=r0: mean(r0) for r0 in rows])
                tasks += _spread(t0 + lag, step, [lambda r0=r0: scale(r0) for r0 in rows])
                tasks += _spread(t0 + 2 * lag + step / 2, step, [lambda r=r, t=t: terms(r, t) for t in range(4)])
            return tasks

        def project_in(slot, u0, dst):
            for c in range(3):
                for r in range(0, HL, 128):
                    def product(i):
                        lhs = _halves(xs[slot, i, _word_rows(r, 128), :])
                        return _dot(lhs, _halves(weaver.operand(wst[u0 + c, i])))

                    def emit(bi, bj, val):
                        for k in (0, 64):
                            dst[c][zw + bj, pl.ds(_token(bi, r + k), 64), :] = val[k:k + 64]

                    yield from _strassen(product, emit)

        def project_out(w, u0, stage_output):
            for r in range(0, HL, 64):
                for v in range(4):
                    def product(i):
                        lhs = jnp.concatenate([os_[t, i, r:r + 64, :] for t in range(NPAIR)], axis=1)
                        return _dot(lhs, _halves(weaver.operand(w[u0 + v, i])))

                    def emit(bi, bj, val):
                        rows = pl.ds(_token(bi, r), 64)
                        y = xres[s, rows, _blk(2 * v + bj)] + val
                        xres[s, rows, _blk(2 * v + bj)] = y
                        if stage_output:
                            xio[s, rows, _blk(2 * v + bj)] = y.astype(BF16)

                    yield from _strassen(product, emit)

        def put_heads(p, r):
            top, bot = pl.ds(_token(0, r), 32), pl.ds(_token(1, r), 32)
            terms = _lhs_terms(paced(otmp[0][zr, top]), otmp[1][zr, top],
                               otmp[0][zr, bot], paced(otmp[1][zr, bot]))
            for i, term in enumerate(terms):
                os_[p + zr, i, r:r + 32, :] = term.astype(BF16)

        def attention_a(src, p, e, plan, ready):
            g = 2 * p + e
            kb, vt, qt, fq = abuf[e]
            st = {}

            def prepare_q(i):
                q = weaver.transposed(src[0][zr + e, _blk(i), :])
                turned = [pltpu.roll(q[_blk(h, DH)], DH * h, 1) if h else q[:DH] for h in range(4)]
                qt[zw, i] = _words(jnp.concatenate(turned, axis=0) * QSCALE)
                fq[zw, i] = _words(_phi(q))

            def prepare_k(i):
                kb[zw, i] = _words(paced(src[1][zr + e, _blk(i), :]))

            def prepare_v(i):
                vt[zw, i] = _words(weaver.transposed(src[2][zr + e, _blk(i), :]))

            def whole(buf):
                return _halves(jnp.concatenate([buf[zr, i] for i in range(4)], axis=1))

            def retrieve():
                st["m"] = jnp.where(s > 0, mem[g], 0.0)
                st["nd"] = _dot(st["m"].astype(BF16), whole(fq))

            def features(i):
                fk = _phi(paced(src[1][zr + e, _blk(i), :]))
                st["z"] = _fold(jnp.add, st.get("z"), fk)
                st["fk", i] = fk.astype(BF16)

            def update():
                head = _iota((128, 128), 1) // DH
                upd = _dot(whole(vt), jnp.concatenate([st["fk", i] for i in range(4)], axis=0))
                z = jnp.sum(st["z"], axis=0, keepdims=True)
                mem[g, :128, :] = st["m"][:128] + jnp.where(_iota((128, 128), 0) // DH == head, upd, 0.0)
                mem[g, 128:, :] = st["m"][128:] + jnp.where(_iota((16, 128), 0) == head[:16], z, 0.0)

            def close_max(i):
                mx = _reduce4(jnp.maximum, [st["mx", i, h] for h in range(4)])
                for h in range(4):
                    st["mx", i, h] = jnp.broadcast_to(mx[h:h + 1], (8, 128))
                for c, mx in enumerate(_regroup([st["mx", i, h] for h in range(4)])):
                    st["dmx", i, c] = mx

            def qk_diagonal(c):
                keep = (_iota((64, 128), 1) // DH - _iota((64, 128), 0) // 16) % 4 == c
                nk = DH * (c + 1)
                for i in range(4):
                    sc = _dot(_halves(kb[zr, i, :nk // 2, :]), _halves(jnp.where(keep, qt[zr, i], 0)))
                    last = sc[nk - DH:] + cmask[...]
                    sc = jnp.concatenate([sc[:nk - DH], last], axis=0) if c else last
                    sbuf[e][0][zw, i, c, :nk, :] = sc
                    st["dmx", i, c] = _fold(jnp.maximum, None, sc)

            def open_max():
                for i in range(4):
                    for h, mx in enumerate(_regroup([st["dmx", i, c] for c in range(4)])):
                        st["mx", i, h] = mx
                close_max(0)

            def qk(i, j):
                q = qt[zr, i]
                zero = jnp.zeros((16, 128), I32)
                w = jnp.concatenate(
                    [jnp.concatenate([q[_blk(h, 16)] if hh == h else zero for hh in range(4)], axis=0)
                     for h in range(4)], axis=1)
                sc = _dot(_halves(kb[zr, j]), _halves(w))
                for h in range(4):
                    sbuf[e][i][zw, j, h] = sc[:, _blk(h)]
                    st["mx", i, h] = _fold(jnp.maximum, st["mx", i, h], sc[:, _blk(h)])
                if j == i - 1:
                    close_max(i)

            def exponentiate(i, j, k):
                if j < i:
                    pr = jnp.exp2(sbuf[e][i][zr, j, k] - jnp.tile(paced(st["mx", i, k]), (16, 1)))
                    st["l", i, k] = _fold(jnp.add, st.get(("l", i, k)), pr)
                    st["p", i, j, k] = [pr.astype(BF16)]
                    return
                prs = [None] * 4
                for c in range(k, 4):
                    sc = sbuf[e][0][zr, i, c, _blk(k, DH), :]
                    prs[c] = jnp.exp2(sc - jnp.tile(paced(st["dmx", i, c]), (4, 1)))
                    st["dl", i, c] = _fold(jnp.add, st.get(("dl", i, c)), prs[c])
                for h, pr in enumerate(_regroup(prs)):
                    st.setdefault(("p", i, j, h), []).append(pr.astype(BF16))

            def pv(i, j):
                for h in range(4):
                    pr = jnp.concatenate(st.pop(("p", i, j, h)), axis=0)
                    a = _dot(_halves(vt[zr, j, _blk(h, 16), :]), pr)
                    st["a", i, h] = a if j == 0 else st["a", i, h] + a

            def finish(i):
                sums = _regroup([st["dl", i, c] for c in range(4)])
                sums = _reduce4(jnp.add, [x + st["l", i, h] if i else x for h, x in enumerate(sums)])
                local = (1.0 - gate[g]) / sums
                memory = gate[g] / (st["nd"][128:136, _blk(i)] + 1e-6)
                outs = []
                for h in range(4):
                    a = st["a", i, h] * local[h:h + 1]
                    outs.append(st["nd"][_blk(h, DH), _blk(i)] * memory[h:h + 1]
                                + (pltpu.roll(a, 128 - DH * h, 1) if h else a))
                out = jnp.concatenate(outs, axis=0).T
                otmp[e][zw, _blk(i), :] = out
                weaver.due(out)

            t0 = plan["start"]
            tasks = []
            for c, fn in enumerate((prepare_q, prepare_k, prepare_v)):
                tasks += _spread(max(t0 + plan["qkv"[c]], ready[c]), plan["qkv_len"],
                                 [lambda i=i, fn=fn: fn(i) for i in range(4)])
            tasks.append((t0 + plan["retrieve"], retrieve))
            tasks.append((t0 + plan["update"], update))
            tasks += [(t0 + plan["update"] - plan["feat_lead"] - (3 - i) * plan["feat_step"],
                       lambda i=i: features(i)) for i in range(4)]
            tasks += _spread(t0, plan["diag_len"], [lambda c=c: qk_diagonal(c) for c in (3, 2, 1, 0)] + [open_max])
            tq = t0 + plan["diag_len"]
            closed = {0: tq}
            for i in range(4):
                for j in range(i):
                    tasks.append((tq, lambda i=i, j=j: qk(i, j)))
                    closed[i] = tq
                    tq += plan["qk_step"]
            te = -math.inf
            for i in range(4):
                for j in range(i + 1):
                    te = max(te + plan["exp_step"], closed[i] + plan["exp_lag"])
                    tasks += _spread(te, plan["exp_step"],
                                     [lambda i=i, j=j, k=k: exponentiate(i, j, k) for k in range(4)])
                    tasks.append((te + plan["pv_lag"], lambda i=i, j=j: pv(i, j)))
                tf = max(te + plan["pv_lag"], t0 + plan["retrieve"]) + plan["finish_lag"]
                tasks.append((tf, lambda i=i: finish(i)))
                if e == 1:
                    tasks += [(tf + plan["put_lag"] + k * plan["put_step"],
                               lambda r=64 * i + 32 * k: put_heads(p, r)) for k in range(2)]
            return tasks

        def attention_b(src, p, e, plan, ready):
            g = 2 * p + e
            st = {}

            def bits(t):
                return lax.bitcast_convert_type(t.astype(BF16).astype(F32), I32)

            def pack(r):
                if r == 0:
                    kvn[e][zw, :HALO, :] = jnp.where(s > 0, halo[g], 0)
                sixteen = weaver.constant(16, 32)
                kv = bits(src[1][zr + e, r:r + 32, :]) | lax.shift_right_logical(
                    bits(src[2][zr + e, r:r + 32, :]), sixteen)
                kvn[e][zw, HALO + r:HALO + r + 32, :] = kv
                if r + 32 == L:
                    halo[g] = kv[32 - HALO:]

            def flip(par, t):
                if t < 9:
                    x = kvn[e][zr, pl.ds(HALO + par + 2 * t - 14, 128, stride=4), :]
                else:
                    x = lax.bitcast_convert_type(src[0][zr + e, pl.ds(par + 2 * (t - 9), 128, stride=4), :], I32)
                kvt[e][par][zw, t] = weaver.transposed(x)

            def score(par, h, t):
                high = weaver.constant(-65536, DH)
                k = lax.bitcast_convert_type(kvt[e][par][zr, t, _blk(h, DH), :] & high, F32)
                for a in range(2):
                    w = 7 + a - t
                    if 0 <= w < WIN:
                        x = lax.bitcast_convert_type(kvt[e][par][(3 + t) * zr, 9 + a, _blk(h, DH), :], F32) * k
                        x = (x[0:8] + x[8:16]) + (x[16:24] + x[24:32])
                        sh = 1
                        while (4 * a + h) & sh:
                            x = _merge(jnp.add, st.pop(("part", par, w, sh)), x, sh)
                            sh *= 2
                        st["part", par, w, sh] = x

            def softmax(par):
                token = s * L + 4 * _iota((8, 128), 1) + par + 2 * (_iota((8, 128), 0) // 4)
                lg = [paced(st.pop(("part", par, w, 8))) * QSCALE for w in range(WIN)]
                lg = [jnp.where(token >= DIL * w, x, NEG) for w, x in enumerate(lg)]
                mx = _tree(jnp.maximum, lg)
                pr = [jnp.exp2(x - mx) for x in lg]
                inv = 1.0 / _tree(jnp.add, pr)
                st["p", par] = [x * inv for x in pr]

            def mix(par, h, t):
                sixteen = weaver.constant(16, DH)
                v = lax.bitcast_convert_type(kvt[e][par][2 * zr, t, _blk(h, DH), :] << sixteen, F32)
                for a in range(2):
                    w = 7 + a - t
                    if 0 <= w < WIN:
                        x = st["p", par][w][4 * a + h:4 * a + h + 1] * v
                        st["acc", par, a] = x if w == WIN - 1 else st["acc", par, a] + x
                    if w == 0:
                        otr[e][par][zw, a, _blk(h, DH), :] = st["acc", par, a]

            def unflip(par, a):
                otmp[e][zw, pl.ds(par + 2 * a, 128, stride=4), :] = weaver.transposed(otr[e][par][zr, a])

            t0 = plan["start"]
            tasks = _spread(max(t0 + plan["pack"], ready[2]), plan["pack_len"],
                            [lambda r=r: pack(r) for r in range(0, L, 32)])
            score_len = plan["parity_len"] * plan["score_part"]
            mix_len = plan["parity_len"] * (1 - plan["score_part"])
            for par in range(2):
                tasks += _spread(t0 + plan["flip%d" % par], plan["flip_len"],
                                 [lambda par=par, t=t: flip(par, t) for t in (9, 10, *range(9))])
                tp = t0 + plan["score"] + par * plan["parity_len"]
                tasks += _spread(tp, score_len, [lambda par=par, h=h, t=t: score(par, h, t)
                                                 for t in range(9) for h in range(4)])
                tp = tp + score_len + 0.5
                tasks.append((tp, lambda par=par: softmax(par)))
                tasks += _spread(tp + 0.5, mix_len, [lambda par=par, h=h, t=t: mix(par, h, t)
                                                     for h in range(4) for t in range(9)])
                tp += 0.5 + mix_len
                tasks += [(tp + plan["unflip_lag"], lambda par=par, a=a: unflip(par, a)) for a in range(2)]
            if e == 1:
                tasks += [(plan["put"] + k * plan["put_step"], lambda r=32 * k: put_heads(p, r)) for k in range(8)]
            return tasks

        def pairs(attention, plans, first, count):
            projections, tasks = [], []
            for j in range(count):
                p = first + j
                nxt = n + (p + 1) // NPAIR
                u0 = ((nxt // NSEG) % 2) * NUNIT + ((p + 1) % NPAIR) * 3
                ready = [STEP * (j - 1) + STEP // 3 * (c + 1) - 0.01 if j else -1 for c in range(3)]
                for e in range(2):
                    plan = {name: column[2 * j + e] for name, column in plans.items()}
                    tasks += attention(qkv[j % 2], p, e, plan, ready)
                projections.append(project_in(nxt % 2, u0, qkv[(j + 1) % 2]))
            return projections, tasks

        @pl.when(n == 0)
        def _():
            def arrive(i):
                x0_copy(i).wait()
                if i == 1:
                    x_copy(1).start()
                else:
                    fetch(*{0: (1, 3), 2: (3, 6), 3: (6, 9)}[i])

            weaver.run((), [(4 * i - 0.5, lambda i=i: arrive(i)) for i in range(4)]
                       + layernorm(0, 0, 0, 1, 1, from_input=True))
            prepare_weights(0, 1)
            tasks = [(12, x_copy(1).wait)] + layernorm(1, 1, 12, 25 / 16, 1.5, from_input=True)
            for u, t in ((1, 2), (2, 7)):
                tasks += [(t, w_copy(u).wait)] + _spread(t, 5, weight_terms(u))
            weaver.run([project_in(0, 0, qkv[0])], tasks)

        @pl.when(kind == 0)
        def _():
            def fetch_more(u):
                @pl.when(u == 8)
                def _():
                    fetch(9, 20)
                    x_copy(2).start()
                    x_copy(3).start()

            def widen(u):
                rows = pl.ds(pl.multiple_of(u % 2 * HL, HL), HL)
                xres[u // 2 - 4, rows, :] = xio[u // 2 - 4, rows, :].astype(F32)

            def half(it, carry):
                lo = 3 + 6 * it
                prepare_weights(lo, jnp.where(n == 0, 9 + 3 * it, lo), fetch_more)
                weaver.run(*pairs(attention_a, PLAN_A, 2 * it, 2))
                return carry

            lax.fori_loop(0, 2, half, 0)

            @pl.when(n == 0)
            def _():
                fetch(20, 2 * NUNIT)
                x_copy(2).wait()
                x_copy(3).wait()
                prepare_weights(12, NUNIT, widen, wsa, 12)

            @pl.when(n < NSEG)
            def _():
                for k in range(4):
                    u = NUNIT + 4 * n + k
                    pltpu.make_async_copy(wraw.at[u], wraw.at[u], wsem.at[u]).wait()

            tasks = layernorm((n + 2) % NSEG, n % 2, -1, 6.6, 3)
            tasks += _spread(0, 111, [f for k in range(4) for f in weight_terms(NUNIT + 4 * s + k)])
            weaver.run([project_out(wsa, 0, False)], tasks)

        @pl.when(kind == 1)
        def _():
            def send(i):
                pl.when(n >= 3 * NSEG)(lambda: out_copy(s, i).start())

            projections, tasks = pairs(attention_b, PLAN_B, 0, NPAIR)
            tasks += layernorm((n + 2) % NSEG, n % 2, STEP * NPAIR, 6, 3)
            tasks += [(STEP * NPAIR + 28 * (i + 1) + 3, lambda i=i: send(i)) for i in range(4)]
            weaver.run(projections + [project_out(wst, NUNIT + 12, True)], tasks)

        return carry

    lax.fori_loop(0, 4 * NSEG, segment, 0)
    for s in range(NSEG):
        for i in range(4):
            out_copy(s, i).wait()


def _call(**kwargs):
    hbm = pl.BlockSpec(memory_space=pl.ANY)
    return pl.pallas_call(
        _kernel,
        out_shape=jax.ShapeDtypeStruct((S, D), BF16),
        in_specs=[hbm] * 8,
        out_specs=hbm,
        scratch_shapes=[
            pltpu.VMEM((NSEG, L, D), BF16),
            pltpu.VMEM((NSEG, L, D), F32),
            pltpu.VMEM((1, L, D), F32),
            pltpu.VMEM((2, 7, HL // 2, D // 2), I32),
            pltpu.VMEM((NPAIR, 7, HL, 128), BF16),
            pltpu.VMEM((2 * NUNIT, D, 256), BF16),
            pltpu.VMEM((2 * NUNIT, 7, 256, 128), I32),
            pltpu.VMEM((4, 7, 256, 128), I32),
            pltpu.VMEM((2 * NPAIR, 144, 128), F32),
            pltpu.VMEM((2 * NPAIR, 8, 128), F32),
            pltpu.VMEM((DH, 128), F32),
            pltpu.VMEM((2 * NPAIR, HALO, 128), I32),
            pltpu.SemaphoreType.DMA((NSEG + 3,)),
            pltpu.SemaphoreType.DMA((2 * NUNIT,)),
            pltpu.SemaphoreType.DMA((4 * NSEG,)),
            pltpu.SemaphoreType.DMA(()),
        ]
        + [pltpu.VMEM((1, HALO + L + PAD, 128), I32)] * 2
        + [pltpu.VMEM((1, L + PAD, 128), F32)] * 2
        + [pltpu.VMEM((2, L + PAD, 128), F32)] * 6
        + [pltpu.VMEM((1, 4, 64, 128), I32)] * 8
        + [pltpu.VMEM((1, i or 4, 4, 128, 128), F32) for i in range(4)] * 2
        + [pltpu.VMEM((1, 11, 128, 128), I32)] * 4
        + [pltpu.VMEM((1, 2, 128, 128), F32)] * 4
        + [pltpu.VMEM((1, H), BF16)],
        compiler_params=pltpu.CompilerParams(vmem_limit_bytes=110 * 2 ** 20),
        name="fused",
        **kwargs,
    )


@jax.jit
def pallas_interleave_layers__memory_aug_infini_attn__sliding_local_dilated__prompt_kernel(
    A_x: jax.Array,
    A_wq: jax.Array,
    A_wk: jax.Array,
    A_wv: jax.Array,
    A_wo: jax.Array,
    A_beta: jax.Array,
    B_x: jax.Array,
    B_wqkv: jax.Array,
    B_wo: jax.Array,
):
    del B_x
    out = _call()(A_x.reshape(S, D), A_wq, A_wk, A_wv, A_wo, A_beta.reshape(1, H), B_wqkv, B_wo)
    return out.reshape(A_x.shape)
```

```python
import math

import jax
import jax.numpy as jnp
from jax import lax
import jax.experimental.pallas as pl
import jax.experimental.pallas.tpu as pltpu

S, D, H, DH = 2048, 1024, 32, 32
NSEG, L = 4, 512
HL = L // 2
NPAIR = 4
NUNIT = 16
STEP = 42
WIN, DIL = 8, 2
HALO = 16
PAD = 32
LOG2E = math.log2(math.e)
QSCALE = DH ** -0.5 * LOG2E
NEG = -1e9 * LOG2E
F32, BF16, I32 = jnp.float32, jnp.bfloat16, jnp.int32

PLAN_A = dict(
    start=(5, 22, 40.5, 58.5), q=(-6.7, -6.3, -6.6, -6.3), k=(-6, -3, -2.3, -4),
    v=(-1.4, -3.7, -2, -2.6), qkv_len=(2, 2, 1.7, 1.1), retrieve=(3.7, 4.3, 3.7, 1.7),
    update=(12.3, 13.3, 12.3, 12.3), feat_lead=(1.5, 3.1, 0.6, 0.9), feat_step=(0.6, 0.7, 0.8, 0.6),
    diag_len=(2.5,) * 4, qk_step=(2, 2.2, 1.95, 2.05), exp_step=(1.7, 1.7, 1.6, 1.5),
    exp_lag=(1.5, 0.5, 1.5, 1.2), pv_lag=(2.8, 2.5, 2.8, 2.8), finish_lag=(0.4, 1, 1, 1.6),
    put_lag=(0, 3, 0, 0.8), put_step=(0, 0.95, 0, 0.83))
PLAN_B = dict(
    start=(-1.6, 17.7, 41.4, 60.1, 83.4, 101.7, 125.4, 139.4), pack=(-0.2, -6, 0, -6, -0.3, -6, 0, -6),
    pack_len=(1, 2.3, 1, 3, 1, 2.6, 1, 3), flip0=(1, -2) * 4, flip1=(7, 6.4, 7, 6.4, 7, 6.4, 7, 7.6),
    flip_len=(3.3, 3.8, 4, 4, 4, 4, 4.2, 4), score=(6.5, 4, 6.7, 4, 6.5, 4, 8.5, 4),
    parity_len=(9, 9, 9, 9, 9.2, 9, 7.3, 8.4), score_part=(0.62, 0.62, 0.62, 0.62, 0.74, 0.62, 0.62, 0.62),
    unflip_lag=(0.8, 1.2, 1.2, 1.2, 1.2, 1.2, 1.2, 0.6),
    put=(0, 44, 0, 86, 0, 127.8, 0, 162.9), put_step=(0, 0.2, 0, 0.2, 0, 0.32, 0, 0.08))


def _dot(a, b):
    return jnp.dot(a, b, preferred_element_type=F32)


def _iota(shape, axis):
    return lax.broadcasted_iota(I32, shape, axis)


def _words(x):
    return pltpu.bitcast(x.astype(BF16), I32)


def _halves(x):
    return pltpu.bitcast(x, BF16)


def _word_rows(start, size):
    return slice(start // 2, (start + size) // 2)


def _blk(i, n=128):
    return slice(i * n, (i + 1) * n)


def _token(half, r):
    return r // 64 * 128 + half * 64 + r % 64


def _phi(t):
    return jnp.where(t > 0, t + 1.0, jnp.exp(t))


def _lhs_terms(a11, a12, a21, a22):
    return (a11 + a22, a21 + a22, a11, a22, a11 + a12, a21 - a11, a12 - a22)


def _strassen(product, emit):
    m = product(0)
    c11 = c22 = m
    yield m
    m = product(6)
    c11 = c11 + m
    yield m
    m = product(5)
    c22 = c22 + m
    yield m
    c21 = product(3)
    c11 = c11 + c21
    yield c21
    m = product(1)
    c22 = c22 - m
    emit(1, 0, c21 + m)
    yield m
    c12 = product(4)
    emit(0, 0, c11 - c12)
    yield c12
    m = product(2)
    emit(1, 1, c22 + m)
    emit(0, 1, c12 + m)
    yield m


def _regroup(xs):
    lane = _iota(xs[3].shape, 1)

    def pick(bit, one, zero):
        if one is None and zero is None:
            return None
        return jnp.where((lane & bit) != 0, 0.0 if one is None else one, 0.0 if zero is None else zero)

    us = [pick(32, xs[(a + 1) % 4], xs[a]) for a in range(4)]
    return [pick(64, us[(2 - a) % 4], us[-a % 4]) for a in range(4)]


def _merge(op, x, y, sh):
    bit = (_iota((8, 128), 0) & sh) != 0
    return op(jnp.where(bit, y, x), pltpu.roll(jnp.where(bit, x, y), sh, 0))


def _reduce4(op, xs):
    t = _merge(op, _merge(op, xs[0], xs[1], 1), _merge(op, xs[2], xs[3], 1), 2)
    return op(t, pltpu.roll(t, 4, 0))


def _tree(op, xs):
    while len(xs) > 1:
        xs = [op(a, b) for a, b in zip(xs[0::2], xs[1::2])]
    return xs[0]


def _fold(op, acc, x):
    for r in range(0, x.shape[0], 8):
        acc = x[r:r + 8] if acc is None else op(acc, x[r:r + 8])
    return acc


def _spread(start, length, thunks):
    return [(start + length * k / len(thunks), f) for k, f in enumerate(thunks)]


class _Weaver:
    def __init__(self, never):
        self.never = never
        self.rows, self.count, self.waits = None, 0, {}

    def run(self, projections, tasks):
        tasks = sorted(tasks, key=lambda t: t[0])
        k = 0
        while k < len(tasks) and tasks[k][0] < 0:
            tasks[k][1]()
            k += 1
        for i, m in enumerate(m for products in projections for m in products):
            while k < len(tasks) and tasks[k][0] < i + 1:
                r = int((tasks[k][0] - i) * m.shape[0]) // 8 * 8
                self.rows = m[r:r + 8]
                tasks[k][1]()
                k += 1
        for _, thunk in tasks[k:]:
            thunk()
        self.rows, self.count, self.waits = None, 0, {}

    def paced(self, x):
        if self.rows is None:
            return x
        rows = lax.bitcast_convert_type(self.rows, x.dtype)
        return jnp.where(self.never, jnp.tile(rows, (x.shape[0] // 8, 1)), x)

    def transposed(self, x):
        return jnp.concatenate([self.paced(x[:8]), x[8:]], axis=0).T

    def constant(self, value, rows):
        return jnp.tile(self.paced(jnp.full((8, 128), value, I32)), (rows // 8, 1))

    def due(self, x):
        self.waits[self.count + 4] = x[-8:]

    def operand(self, w):
        head = w[:8]
        if self.count in self.waits:
            head = jnp.where(self.never, lax.bitcast_convert_type(self.waits.pop(self.count), I32), head)
        self.count += 1
        return jnp.concatenate([head, w[8:]], axis=0)


def _kernel(x_hbm, wq_hbm, wk_hbm, wv_hbm, woa_hbm, beta_hbm, wqkv_hbm, wob_hbm, out_hbm,
            xio, xres, xtmp, xs, os_, wraw, wst, wsa, mem, gate, cmask, halo, xsem, wsem, osem, bsem, *bufs):
    *bufs, beta_ref = bufs
    kvn, otmp = ([bufs.pop(0) for _ in range(2)] for _ in range(2))
    qkv, abuf, sbuf, kvt, otr = (
        [[bufs.pop(0) for _ in range(k)] for _ in range(2)] for k in (3, 4, 4, 2, 2))

    def x0_copy(i):
        return pltpu.make_async_copy(x_hbm.at[_blk(i)], xio.at[0, _blk(i)], xsem.at[i])

    def x_copy(s):
        rows = pl.ds(pl.multiple_of(s * L, L), L)
        return pltpu.make_async_copy(x_hbm.at[rows], xio.at[s], xsem.at[s + 3])

    def w_copy(u):
        kind, v = divmod(u, NUNIT)
        if v >= 12:
            src, col = (woa_hbm, wob_hbm)[kind], (v - 12) * 256
        elif kind == 0:
            src, col = (wq_hbm, wk_hbm, wv_hbm)[v % 3], (v // 3) * 256
        else:
            src, col = wqkv_hbm, (v % 3) * D + (v // 3) * 256
        return pltpu.make_async_copy(src.at[:, pl.ds(col, 256)], wraw.at[u], wsem.at[u])

    def out_copy(s, i):
        rows = pl.ds(pl.multiple_of(s * L + i * 128, 128), 128)
        return pltpu.make_async_copy(xio.at[s, _blk(i)], out_hbm.at[rows], osem.at[4 * s + i])

    def fetch(lo, hi):
        for u in range(lo, hi):
            w_copy(u).start()

    beta_copy = pltpu.make_async_copy(beta_hbm, beta_ref, bsem)
    beta_copy.start()
    for i in range(4):
        x0_copy(i).start()
    fetch(0, 1)
    beta_copy.wait()

    row = _iota((64, H), 0)
    beta = jnp.broadcast_to(beta_ref[...].astype(F32), (64, H))
    beta = jnp.sum(jnp.where(row // 8 * 4 + row % 4 == _iota((64, H), 1), beta, 0.0), axis=1, keepdims=True)
    gate[...] = jnp.broadcast_to(1.0 / (1.0 + jnp.exp(-beta)), (64, 128)).reshape(8, 8, 128)
    cmask[...] = jnp.where(_iota((DH, 128), 0) <= _iota((DH, 128), 1) % DH, 0.0, NEG)

    def segment(n, carry):
        kind = (n // NSEG) % 2
        s = n % NSEG
        zr = lax.shift_right_logical(n, 8)
        zw = lax.shift_right_logical(n, 9)
        weaver = _Weaver(zr > 0)
        paced = weaver.paced

        def weight_terms(u, dst=wst, first=0):
            def rows(t, r):
                top = wraw[u, 256 * t + r:256 * t + r + 16, :]
                bot = wraw[u, 256 * t + 128 + r:256 * t + 128 + r + 16, :]
                b1, b2 = top.astype(F32), bot.astype(F32)
                b11, b12, b21, b22 = paced(b1[:, :128]), b1[:, 128:], b2[:, :128], paced(b2[:, 128:])
                sums = _words(jnp.concatenate((b11 + b22, b12 - b22, b21 - b11, b11 + b12, b21 + b22), axis=1))
                sums = [sums[:, _blk(i)] for i in range(5)]
                terms = (sums[0], paced(_words(top[:, :128])), sums[1], sums[2], paced(_words(bot[:, 128:])),
                         sums[3], sums[4])
                for i, term in enumerate(terms):
                    dst[u - first, i, _word_rows(128 * t + r, 16), :] = term

            return [lambda t=t, r=r: rows(t, r) for t in range(4) for r in range(0, 128, 16)]

        def prepare_weights(lo, hi, also=lambda u: None, *where):
            def body(u, carry):
                pltpu.make_async_copy(wraw.at[u], wraw.at[u], wsem.at[u]).wait()
                also(u)
                for thunk in weight_terms(u, *where):
                    thunk()
                return carry

            lax.fori_loop(lo, hi, body, 0)

        def layernorm(sn, slot, start, step, lag, from_input=False):
            st = {}

            def mean(r):
                if from_input:
                    x = xio[sn, r:r + 16, :].astype(F32)
                    xres[sn, r:r + 16, :] = x
                else:
                    x = xres[sn, r:r + 16, :]
                xtmp[3 * zr, r:r + 16, :] = x
                acc = paced(x[:, :128])
                for t in range(1, 8):
                    acc = acc + x[:, _blk(t)]
                st["m", r] = jnp.broadcast_to(jnp.sum(acc, axis=1, keepdims=True) * (1.0 / D), (16, 128))

            def scale(r):
                m = paced(st["m", r])
                acc = None
                for t in range(8):
                    c = xtmp[zr, r:r + 16, _blk(t)] - m
                    acc = c * c if acc is None else acc + c * c
                var = jnp.sum(acc, axis=1, keepdims=True) * (1.0 / D)
                st["r", r] = jnp.broadcast_to(lax.rsqrt(var + 1e-5), (16, 128))

            def terms(r, t):
                ys = []
                for r0 in (_token(0, r), _token(1, r)):
                    m = paced(st["m", r0])
                    ys += [(xtmp[2 * zr, r0:r0 + 16, _blk(2 * t + k)] - m) * st["r", r0] for k in range(2)]
                words = _words(jnp.concatenate(_lhs_terms(*ys), axis=1))
                for i in range(7):
                    xs[slot, i, _word_rows(r, 16), _blk(t)] = words[:, _blk(i)]
                weaver.due(words[:, _blk(6)])

            tasks = []
            for k, r in enumerate(range(0, HL, 16)):
                t0 = start + k * step
                rows = (_token(0, r), _token(1, r))
                tasks += _spread(t0, step, [lambda r0=r0: mean(r0) for r0 in rows])
                tasks += _spread(t0 + lag, step, [lambda r0=r0: scale(r0) for r0 in rows])
                tasks += _spread(t0 + 2 * lag + step / 2, step, [lambda r=r, t=t: terms(r, t) for t in range(4)])
            return tasks

        def project_in(slot, u0, dst):
            for c in range(3):
                for r in range(0, HL, 128):
                    def product(i):
                        lhs = _halves(xs[slot, i, _word_rows(r, 128), :])
                        return _dot(lhs, _halves(weaver.operand(wst[u0 + c, i])))

                    def emit(bi, bj, val):
                        for k in (0, 64):
                            dst[c][zw + bj, pl.ds(_token(bi, r + k), 64), :] = val[k:k + 64]

                    yield from _strassen(product, emit)

        def project_out(w, u0, stage_output):
            for r in range(0, HL, 64):
                for v in range(4):
                    def product(i):
                        lhs = jnp.concatenate([os_[t, i, r:r + 64, :] for t in range(NPAIR)], axis=1)
                        return _dot(lhs, _halves(weaver.operand(w[u0 + v, i])))

                    def emit(bi, bj, val):
                        rows = pl.ds(_token(bi, r), 64)
                        y = xres[s, rows, _blk(2 * v + bj)] + val
                        xres[s, rows, _blk(2 * v + bj)] = y
                        if stage_output:
                            xio[s, rows, _blk(2 * v + bj)] = y.astype(BF16)

                    yield from _strassen(product, emit)

        def put_heads(p, r):
            top, bot = pl.ds(_token(0, r), 32), pl.ds(_token(1, r), 32)
            terms = _lhs_terms(paced(otmp[0][zr, top]), otmp[1][zr, top],
                               otmp[0][zr, bot], paced(otmp[1][zr, bot]))
            for i, term in enumerate(terms):
                os_[p + zr, i, r:r + 32, :] = term.astype(BF16)

        def attention_a(src, p, e, plan, ready):
            g = 2 * p + e
            kb, vt, qt, fq = abuf[e]
            st = {}

            def prepare_q(i):
                q = weaver.transposed(src[0][zr + e, _blk(i), :])
                turned = [pltpu.roll(q[_blk(h, DH)], DH * h, 1) if h else q[:DH] for h in range(4)]
                qt[zw, i] = _words(jnp.concatenate(turned, axis=0) * QSCALE)
                fq[zw, i] = _words(_phi(q))

            def prepare_k(i):
                kb[zw, i] = _words(paced(src[1][zr + e, _blk(i), :]))

            def prepare_v(i):
                vt[zw, i] = _words(weaver.transposed(src[2][zr + e, _blk(i), :]))

            def whole(buf):
                return _halves(jnp.concatenate([buf[zr, i] for i in range(4)], axis=1))

            def retrieve():
                st["m"] = jnp.where(s > 0, mem[g], 0.0)
                st["nd"] = _dot(st["m"].astype(BF16), whole(fq))

            def features(i):
                fk = _phi(paced(src[1][zr + e, _blk(i), :]))
                st["z"] = _fold(jnp.add, st.get("z"), fk)
                st["fk", i] = fk.astype(BF16)

            def update():
                head = _iota((128, 128), 1) // DH
                upd = _dot(whole(vt), jnp.concatenate([st["fk", i] for i in range(4)], axis=0))
                z = jnp.sum(st["z"], axis=0, keepdims=True)
                mem[g, :128, :] = st["m"][:128] + jnp.where(_iota((128, 128), 0) // DH == head, upd, 0.0)
                mem[g, 128:, :] = st["m"][128:] + jnp.where(_iota((16, 128), 0) == head[:16], z, 0.0)

            def close_max(i):
                mx = _reduce4(jnp.maximum, [st["mx", i, h] for h in range(4)])
                for h in range(4):
                    st["mx", i, h] = jnp.broadcast_to(mx[h:h + 1], (8, 128))
                for c, mx in enumerate(_regroup([st["mx", i, h] for h in range(4)])):
                    st["dmx", i, c] = mx

            def qk_diagonal(c):
                keep = (_iota((64, 128), 1) // DH - _iota((64, 128), 0) // 16) % 4 == c
                nk = DH * (c + 1)
                for i in range(4):
                    sc = _dot(_halves(kb[zr, i, :nk // 2, :]), _halves(jnp.where(keep, qt[zr, i], 0)))
                    last = sc[nk - DH:] + cmask[...]
                    sc = jnp.concatenate([sc[:nk - DH], last], axis=0) if c else last
                    sbuf[e][0][zw, i, c, :nk, :] = sc
                    st["dmx", i, c] = _fold(jnp.maximum, None, sc)

            def open_max():
                for i in range(4):
                    for h, mx in enumerate(_regroup([st["dmx", i, c] for c in range(4)])):
                        st["mx", i, h] = mx
                close_max(0)

            def qk(i, j):
                q = qt[zr, i]
                zero = jnp.zeros((16, 128), I32)
                w = jnp.concatenate(
                    [jnp.concatenate([q[_blk(h, 16)] if hh == h else zero for hh in range(4)], axis=0)
                     for h in range(4)], axis=1)
                sc = _dot(_halves(kb[zr, j]), _halves(w))
                for h in range(4):
                    sbuf[e][i][zw, j, h] = sc[:, _blk(h)]
                    st["mx", i, h] = _fold(jnp.maximum, st["mx", i, h], sc[:, _blk(h)])
                if j == i - 1:
                    close_max(i)

            def exponentiate(i, j, k):
                if j < i:
                    pr = jnp.exp2(sbuf[e][i][zr, j, k] - jnp.tile(paced(st["mx", i, k]), (16, 1)))
                    st["l", i, k] = _fold(jnp.add, st.get(("l", i, k)), pr)
                    st["p", i, j, k] = [pr.astype(BF16)]
                    return
                prs = [None] * 4
                for c in range(k, 4):
                    sc = sbuf[e][0][zr, i, c, _blk(k, DH), :]
                    prs[c] = jnp.exp2(sc - jnp.tile(paced(st["dmx", i, c]), (4, 1)))
                    st["dl", i, c] = _fold(jnp.add, st.get(("dl", i, c)), prs[c])
                for h, pr in enumerate(_regroup(prs)):
                    st.setdefault(("p", i, j, h), []).append(pr.astype(BF16))

            def pv(i, j):
                for h in range(4):
                    pr = jnp.concatenate(st.pop(("p", i, j, h)), axis=0)
                    a = _dot(_halves(vt[zr, j, _blk(h, 16), :]), pr)
                    st["a", i, h] = a if j == 0 else st["a", i, h] + a

            def finish(i):
                sums = _regroup([st["dl", i, c] for c in range(4)])
                sums = _reduce4(jnp.add, [x + st["l", i, h] if i else x for h, x in enumerate(sums)])
                local = (1.0 - gate[g]) / sums
                memory = gate[g] / (st["nd"][128:136, _blk(i)] + 1e-6)
                outs = []
                for h in range(4):
                    a = st["a", i, h] * local[h:h + 1]
                    outs.append(st["nd"][_blk(h, DH), _blk(i)] * memory[h:h + 1]
                                + (pltpu.roll(a, 128 - DH * h, 1) if h else a))
                out = jnp.concatenate(outs, axis=0).T
                otmp[e][zw, _blk(i), :] = out
                weaver.due(out)

            t0 = plan["start"]
            tasks = []
            for c, fn in enumerate((prepare_q, prepare_k, prepare_v)):
                tasks += _spread(max(t0 + plan["qkv"[c]], ready[c]), plan["qkv_len"],
                                 [lambda i=i, fn=fn: fn(i) for i in range(4)])
            tasks.append((t0 + plan["retrieve"], retrieve))
            tasks.append((t0 + plan["update"], update))
            tasks += [(t0 + plan["update"] - plan["feat_lead"] - (3 - i) * plan["feat_step"],
                       lambda i=i: features(i)) for i in range(4)]
            tasks += _spread(t0, plan["diag_len"], [lambda c=c: qk_diagonal(c) for c in (3, 2, 1, 0)] + [open_max])
            tq = t0 + plan["diag_len"]
            closed = {0: tq}
            for i in range(4):
                for j in range(i):
                    tasks.append((tq, lambda i=i, j=j: qk(i, j)))
                    closed[i] = tq
                    tq += plan["qk_step"]
            te = -math.inf
            for i in range(4):
                for j in range(i + 1):
                    te = max(te + plan["exp_step"], closed[i] + plan["exp_lag"])
                    tasks += _spread(te, plan["exp_step"],
                                     [lambda i=i, j=j, k=k: exponentiate(i, j, k) for k in range(4)])
                    tasks.append((te + plan["pv_lag"], lambda i=i, j=j: pv(i, j)))
                tf = max(te + plan["pv_lag"], t0 + plan["retrieve"]) + plan["finish_lag"]
                tasks.append((tf, lambda i=i: finish(i)))
                if e == 1:
                    tasks += [(tf + plan["put_lag"] + k * plan["put_step"],
                               lambda r=64 * i + 32 * k: put_heads(p, r)) for k in range(2)]
            return tasks

        def attention_b(src, p, e, plan, ready):
            g = 2 * p + e
            st = {}

            def bits(t):
                return lax.bitcast_convert_type(t.astype(BF16).astype(F32), I32)

            def pack(r):
                if r == 0:
                    kvn[e][zw, :HALO, :] = jnp.where(s > 0, halo[g], 0)
                sixteen = weaver.constant(16, 32)
                kv = bits(src[1][zr + e, r:r + 32, :]) | lax.shift_right_logical(
                    bits(src[2][zr + e, r:r + 32, :]), sixteen)
                kvn[e][zw, HALO + r:HALO + r + 32, :] = kv
                if r + 32 == L:
                    halo[g] = kv[32 - HALO:]

            def flip(par, t):
                if t < 9:
                    x = kvn[e][zr, pl.ds(HALO + par + 2 * t - 14, 128, stride=4), :]
                else:
                    x = lax.bitcast_convert_type(src[0][zr + e, pl.ds(par + 2 * (t - 9), 128, stride=4), :], I32)
                kvt[e][par][zw, t] = weaver.transposed(x)

            def score(par, h, t):
                high = weaver.constant(-65536, DH)
                k = lax.bitcast_convert_type(kvt[e][par][zr, t, _blk(h, DH), :] & high, F32)
                for a in range(2):
                    w = 7 + a - t
                    if 0 <= w < WIN:
                        x = lax.bitcast_convert_type(kvt[e][par][(3 + t) * zr, 9 + a, _blk(h, DH), :], F32) * k
                        x = (x[0:8] + x[8:16]) + (x[16:24] + x[24:32])
                        sh = 1
                        while (4 * a + h) & sh:
                            x = _merge(jnp.add, st.pop(("part", par, w, sh)), x, sh)
                            sh *= 2
                        st["part", par, w, sh] = x

            def softmax(par):
                token = s * L + 4 * _iota((8, 128), 1) + par + 2 * (_iota((8, 128), 0) // 4)
                lg = [paced(st.pop(("part", par, w, 8))) * QSCALE for w in range(WIN)]
                lg = [jnp.where(token >= DIL * w, x, NEG) for w, x in enumerate(lg)]
                mx = _tree(jnp.maximum, lg)
                pr = [jnp.exp2(x - mx) for x in lg]
                inv = 1.0 / _tree(jnp.add, pr)
                st["p", par] = [x * inv for x in pr]

            def mix(par, h, t):
                sixteen = weaver.constant(16, DH)
                v = lax.bitcast_convert_type(kvt[e][par][2 * zr, t, _blk(h, DH), :] << sixteen, F32)
                for a in range(2):
                    w = 7 + a - t
                    if 0 <= w < WIN:
                        x = st["p", par][w][4 * a + h:4 * a + h + 1] * v
                        st["acc", par, a] = x if w == WIN - 1 else st["acc", par, a] + x
                    if w == 0:
                        otr[e][par][zw, a, _blk(h, DH), :] = st["acc", par, a]

            def unflip(par, a):
                otmp[e][zw, pl.ds(par + 2 * a, 128, stride=4), :] = weaver.transposed(otr[e][par][zr, a])

            t0 = plan["start"]
            tasks = _spread(max(t0 + plan["pack"], ready[2]), plan["pack_len"],
                            [lambda r=r: pack(r) for r in range(0, L, 32)])
            score_len = plan["parity_len"] * plan["score_part"]
            mix_len = plan["parity_len"] * (1 - plan["score_part"])
            for par in range(2):
                tasks += _spread(t0 + plan["flip%d" % par], plan["flip_len"],
                                 [lambda par=par, t=t: flip(par, t) for t in (9, 10, *range(9))])
                tp = t0 + plan["score"] + par * plan["parity_len"]
                tasks += _spread(tp, score_len, [lambda par=par, h=h, t=t: score(par, h, t)
                                                 for t in range(9) for h in range(4)])
                tp = tp + score_len + 0.5
                tasks.append((tp, lambda par=par: softmax(par)))
                tasks += _spread(tp + 0.5, mix_len, [lambda par=par, h=h, t=t: mix(par, h, t)
                                                     for h in range(4) for t in range(9)])
                tp += 0.5 + mix_len
                tasks += [(tp + plan["unflip_lag"], lambda par=par, a=a: unflip(par, a)) for a in range(2)]
            if e == 1:
                tasks += [(plan["put"] + k * plan["put_step"], lambda r=32 * k: put_heads(p, r)) for k in range(8)]
            return tasks

        def pairs(attention, plans, first, count):
            projections, tasks = [], []
            for j in range(count):
                p = first + j
                nxt = n + (p + 1) // NPAIR
                u0 = ((nxt // NSEG) % 2) * NUNIT + ((p + 1) % NPAIR) * 3
                ready = [STEP * (j - 1) + STEP // 3 * (c + 1) - 0.01 if j else -1 for c in range(3)]
                for e in range(2):
                    plan = {name: column[2 * j + e] for name, column in plans.items()}
                    tasks += attention(qkv[j % 2], p, e, plan, ready)
                projections.append(project_in(nxt % 2, u0, qkv[(j + 1) % 2]))
            return projections, tasks

        @pl.when(n == 0)
        def _():
            def arrive(i):
                x0_copy(i).wait()
                if i == 1:
                    x_copy(1).start()
                else:
                    fetch(*{0: (1, 3), 2: (3, 6), 3: (6, 9)}[i])

            weaver.run((), [(4 * i - 0.5, lambda i=i: arrive(i)) for i in range(4)]
                       + layernorm(0, 0, 0, 1, 1, from_input=True))
            prepare_weights(0, 1)
            tasks = [(12, x_copy(1).wait)] + layernorm(1, 1, 12, 25 / 16, 1.5, from_input=True)
            for u, t in ((1, 2), (2, 7)):
                tasks += [(t, w_copy(u).wait)] + _spread(t, 5, weight_terms(u))
            weaver.run([project_in(0, 0, qkv[0])], tasks)

        @pl.when(kind == 0)
        def _():
            def fetch_more(u):
                @pl.when(u == 8)
                def _():
                    fetch(9, 20)
                    x_copy(2).start()
                    x_copy(3).start()

            def widen(u):
                rows = pl.ds(pl.multiple_of(u % 2 * HL, HL), HL)
                xres[u // 2 - 4, rows, :] = xio[u // 2 - 4, rows, :].astype(F32)

            def half(it, carry):
                lo = 3 + 6 * it
                prepare_weights(lo, jnp.where(n == 0, 9 + 3 * it, lo), fetch_more)
                weaver.run(*pairs(attention_a, PLAN_A, 2 * it, 2))
                return carry

            lax.fori_loop(0, 2, half, 0)

            @pl.when(n == 0)
            def _():
                fetch(20, 2 * NUNIT)
                x_copy(2).wait()
                x_copy(3).wait()
                prepare_weights(12, NUNIT, widen, wsa, 12)

            @pl.when(n < NSEG)
            def _():
                for k in range(4):
                    u = NUNIT + 4 * n + k
                    pltpu.make_async_copy(wraw.at[u], wraw.at[u], wsem.at[u]).wait()

            tasks = layernorm((n + 2) % NSEG, n % 2, -1, 6.6, 3)
            tasks += _spread(0, 111, [f for k in range(4) for f in weight_terms(NUNIT + 4 * s + k)])
            weaver.run([project_out(wsa, 0, False)], tasks)

        @pl.when(kind == 1)
        def _():
            def send(i):
                pl.when(n >= 3 * NSEG)(lambda: out_copy(s, i).start())

            projections, tasks = pairs(attention_b, PLAN_B, 0, NPAIR)
            tasks += layernorm((n + 2) % NSEG, n % 2, STEP * NPAIR, 6, 3)
            tasks += [(STEP * NPAIR + 28 * (i + 1) + 3, lambda i=i: send(i)) for i in range(4)]
            weaver.run(projections + [project_out(wst, NUNIT + 12, True)], tasks)

        return carry

    lax.fori_loop(0, 4 * NSEG, segment, 0)
    for s in range(NSEG):
        for i in range(4):
            out_copy(s, i).wait()


def _call(**kwargs):
    hbm = pl.BlockSpec(memory_space=pl.ANY)
    return pl.pallas_call(
        _kernel,
        out_shape=jax.ShapeDtypeStruct((S, D), BF16),
        in_specs=[hbm] * 8,
        out_specs=hbm,
        scratch_shapes=[
            pltpu.VMEM((NSEG, L, D), BF16),
            pltpu.VMEM((NSEG, L, D), F32),
            pltpu.VMEM((1, L, D), F32),
            pltpu.VMEM((2, 7, HL // 2, D // 2), I32),
            pltpu.VMEM((NPAIR, 7, HL, 128), BF16),
            pltpu.VMEM((2 * NUNIT, D, 256), BF16),
            pltpu.VMEM((2 * NUNIT, 7, 256, 128), I32),
            pltpu.VMEM((4, 7, 256, 128), I32),
            pltpu.VMEM((2 * NPAIR, 144, 128), F32),
            pltpu.VMEM((2 * NPAIR, 8, 128), F32),
            pltpu.VMEM((DH, 128), F32),
            pltpu.VMEM((2 * NPAIR, HALO, 128), I32),
            pltpu.SemaphoreType.DMA((NSEG + 3,)),
            pltpu.SemaphoreType.DMA((2 * NUNIT,)),
            pltpu.SemaphoreType.DMA((4 * NSEG,)),
            pltpu.SemaphoreType.DMA(()),
        ]
        + [pltpu.VMEM((1, HALO + L + PAD, 128), I32)] * 2
        + [pltpu.VMEM((1, L + PAD, 128), F32)] * 2
        + [pltpu.VMEM((2, L + PAD, 128), F32)] * 6
        + [pltpu.VMEM((1, 4, 64, 128), I32)] * 8
        + [pltpu.VMEM((1, i or 4, 4, 128, 128), F32) for i in range(4)] * 2
        + [pltpu.VMEM((1, 11, 128, 128), I32)] * 4
        + [pltpu.VMEM((1, 2, 128, 128), F32)] * 4
        + [pltpu.VMEM((1, H), BF16)],
        compiler_params=pltpu.CompilerParams(vmem_limit_bytes=110 * 2 ** 20),
        name="fused",
        **kwargs,
    )


@jax.jit
def pallas_interleave_layers__memory_aug_infini_attn__sliding_local_dilated__prompt_kernel(
    A_x: jax.Array,
    A_wq: jax.Array,
    A_wk: jax.Array,
    A_wv: jax.Array,
    A_wo: jax.Array,
    A_beta: jax.Array,
    B_x: jax.Array,
    B_wqkv: jax.Array,
    B_wo: jax.Array,
):
    del B_x
    out = _call()(A_x.reshape(S, D), A_wq, A_wk, A_wv, A_wo, A_beta.reshape(1, H), B_wqkv, B_wo)
    return out.reshape(A_x.shape)
```
